```python
import jax
import jax.numpy as jnp

def _softmax(x, axis=-1):
    return jax.nn.softmax(x, axis=axis)
def _gelu(x):
    return jax.nn.gelu(x, approximate=True)
def _silu(x):
    return jax.nn.silu(x)
def _sigmoid(x):
    return jax.nn.sigmoid(x)
def _layernorm(x, axis=-1, eps=1e-5):
    m = jnp.mean(x, axis=axis, keepdims=True)
    v = jnp.var(x, axis=axis, keepdims=True)
    return (x - m) / jnp.sqrt(v + eps)
def _scatter_add(tgt, idx, src, axis=0):
    return tgt.at[idx].add(src)
def _segment_sum(src, seg, n):
    return jax.ops.segment_sum(src, seg, n)
class _Rng:
    def __init__(self, key):
        self._k = key
    def _next(self):
        self._k, sub = jax.random.split(self._k)
        return sub
    def normal(self, shape):
        return jax.random.normal(self._next(), shape, dtype=jnp.bfloat16)
    def randint(self, lo, hi, shape):
        return jax.random.randint(self._next(), shape, lo, hi, dtype=jnp.int32)
    def uniform(self, shape, lo=0.0, hi=1.0):
        return jax.random.uniform(self._next(), shape, jnp.bfloat16, lo, hi)
    def permutation(self, n):
        return jax.random.permutation(self._next(), n)


kernel_name = 'gated_mix__linear_attn_block__moe_arch_mod__prompt'

def setup_inputs():
    _rng = _Rng(jax.random.key(int.from_bytes(__import__("os").urandom(4), "little")))
    _w = (lambda a: (lambda t: t.astype(jnp.bfloat16) if jnp.issubdtype(t.dtype, jnp.floating) else t)(jnp.asarray(a)))
    def _A_setup():
        B, S, D = 1, 2048, 1024
        return {
            "x": _w((lambda *s: _rng.normal(s) * 0.05)(B, S, D)),
            "wqkv": _w((lambda *s: _rng.normal(s) * 0.05)(D, 3 * D)),
            "wo": _w((lambda *s: _rng.normal(s) * 0.05)(D, D)),
        }
    _A_in = _A_setup()

    def _B_setup():
        B, S, D, F, C = 1, 2048, 1024, 3584, 1
        return {
            "x": _w((lambda *s: _rng.normal(s) * 0.05)(B, S, D)),
            "w_r": _w((lambda *s: _rng.normal(s) * 0.05)(D)),
            "w_gate": _w((lambda *s: _rng.normal(s) * 0.05)(D, F)),
            "w_up": _w((lambda *s: _rng.normal(s) * 0.05)(D, F)),
            "w_down": _w((lambda *s: _rng.normal(s) * 0.05)(F, D)),
        }
    _B_in = _B_setup()

    return {
        "A_x": _A_in["x"],
        "A_wqkv": _A_in["wqkv"],
        "A_wo": _A_in["wo"],
        "B_x": _B_in["x"],
        "B_w_r": _B_in["w_r"],
        "B_w_gate": _B_in["w_gate"],
        "B_w_up": _B_in["w_up"],
        "B_w_down": _B_in["w_down"],
        "gate_w": _w((lambda *s: _rng.normal(s) * 0.05)(1024)),
    }

def reference(A_x, A_wqkv, A_wo, B_x, B_w_r, B_w_gate, B_w_up, B_w_down, gate_w):
    def _A_ref(x, wqkv, wo):
        B, S, D = x.shape
        H = 32; Dh = D // H
        qkv = (lambda x, *d: x.transpose(*d))((x @ wqkv).reshape(B, S, 3, H, Dh), 2, 0, 3, 1, 4)
        q, k, v = qkv[0], qkv[1], qkv[2]
        phi = lambda t: jnp.where(t > 0, t + 1, jnp.exp(t)) + 1e-6
        pq, pk = phi(q), phi(k)
        kv = jnp.einsum("bhsd,bhse->bhde", pk, v)
        z = jnp.einsum("bhsd->bhd", pk)
        num = jnp.einsum("bhqd,bhde->bhqe", pq, kv)
        den = jnp.einsum("bhqd,bhd->bhq", pq, z)[..., None] + 1e-6
        o = num / den
        return (lambda x, *d: x.transpose(*d))(o, 0, 2, 1, 3).reshape(B, S, D) @ wo

    def _B_ref(x, w_r, w_gate, w_up, w_down):
        B, S, D = x.shape
        C = 1
        r = x @ w_r
        idx = jnp.argsort(-r, axis=-1)[:, :C]
        idx_e = jnp.repeat(idx.reshape(B, C, 1), D, axis=2)
        x_sel = jnp.take_along_axis(x, idx_e, axis=1)
        g = _silu(x_sel @ w_gate)
        u = x_sel @ w_up
        y = (g * u) @ w_down
        r_sel = _sigmoid(jnp.take_along_axis(r, idx, axis=1))
        y = y * r_sel.reshape(B, C, 1)
        b_off = (jnp.arange(B) * S).reshape(B, 1)
        flat_idx = (idx + b_off).reshape(B * C)
        zero = (x * 0.0).reshape(B * S, D)
        upd = _scatter_add(zero, flat_idx, y.reshape(B * C, D), axis=0)
        return x + upd.reshape(B, S, D)

    x = A_x
    g = _sigmoid((x * gate_w).sum(-1, keepdims=True))
    a = _A_ref(x, A_wqkv, A_wo)
    b = _B_ref(x, B_w_r, B_w_gate, B_w_up, B_w_down)
    return g * a + (1 - g) * b
```

```python
import jax
import jax.numpy as jnp
from jax import lax
import jax.experimental.pallas as pl
import jax.experimental.pallas.tpu as pltpu

S, D, F, H = 2048, 1024, 3584, 32
DH = D // H
SB = 512
NB = S // SB
FC = F // NB
f32, bf16 = jnp.float32, jnp.bfloat16


def _phi(t):
    return jnp.where(t > 0, t + 1.0, jnp.exp(t)) + 1e-6


def _rnd(t):
    return t.astype(bf16).astype(f32)


def _col_bcast(row):
    n = row.shape[1]
    return jnp.concatenate(
        [jnp.broadcast_to(row[:, j:j + 128], (128, 128)).T for j in range(0, n, 128)], axis=0)


def _lanes(t, n):
    return jnp.concatenate([t] * n, axis=1)


def _kernel(ax_hbm, wqkv_hbm, wo_hbm, wg_hbm, wu_hbm, wd_hbm, vec_ref, out_hbm,
            x_v, w_v, wt_v, wo_v, wg_v, wu_v, wd_v, pt_v, pn_v, g_v, m_v, gr_v, z_v, xb_v,
            y_v, o_v, sem_x, sem_w, sem_f, sem_o):
    def x_copy(i):
        return pltpu.make_async_copy(ax_hbm.at[pl.ds(i * SB, SB)], x_v.at[pl.ds(i * SB, SB)],
                                     sem_x.at[i])

    def w_copy(j):
        if j == 3:
            return pltpu.make_async_copy(wo_hbm, wo_v, sem_w.at[3])
        return pltpu.make_async_copy(wqkv_hbm.at[:, pl.ds(j * D, D)], w_v.at[j], sem_w.at[j])

    def f_copies(c):
        return (pltpu.make_async_copy(wg_hbm.at[:, pl.ds(c * FC, FC)], wg_v.at[c], sem_f.at[0, c]),
                pltpu.make_async_copy(wu_hbm.at[:, pl.ds(c * FC, FC)], wu_v.at[c], sem_f.at[1, c]),
                pltpu.make_async_copy(wd_hbm.at[pl.ds(c * FC, FC)], wd_v.at[c], sem_f.at[2, c]))

    def o_copy(i):
        return pltpu.make_async_copy(o_v.at[pl.ds(i * SB, SB)], out_hbm.at[pl.ds(i * SB, SB)],
                                     sem_o.at[i])

    w_copy(0).start()
    x_copy(0).start()
    w_copy(0).wait()
    for i in range(1, NB):
        x_copy(i).start()
    w_copy(1).start()
    wt_v[0] = w_v[0].T
    z_v[...] = jnp.zeros_like(z_v)

    for t in range(2):
        def proj(i, c, t=t):
            if t == 0:
                x_copy(i).wait()
                for j in range(1, NB):
                    @pl.when(i == j)
                    def _():
                        for cp in f_copies(j - 1):
                            cp.start()
            else:
                @pl.when(i == 0)
                def _():
                    for cp in f_copies(NB - 1):
                        cp.start()

                @pl.when(i == 1)
                def _():
                    w_copy(2).start()
                    w_copy(3).start()
            rows = pl.ds(pl.multiple_of(i * SB, SB), SB)
            tt = lax.dot_general(wt_v[t], x_v[rows, :], (((1,), (1,)), ((), ())),
                                 preferred_element_type=f32)
            p = _phi(tt).astype(bf16)
            pt_v[t, i] = p
            if t == 1:
                pf = p.astype(f32)
                z_v[...] += sum(pf[:, j:j + 128] for j in range(0, SB, 128))
            gr_v[t, rows, :] = jnp.sum(x_v[rows, :].astype(f32) * vec_ref[t:t + 1, :],
                                       axis=1, keepdims=True)
            return c
        lax.fori_loop(0, NB, proj, 0)
        if t == 0:
            w_copy(1).wait()
            wt_v[1] = w_v[1].T

    r = _rnd(gr_v[1])
    r_max = jnp.max(r, axis=0, keepdims=True)
    tok = lax.broadcasted_iota(jnp.int32, (S, 1), 0)
    idx = jnp.min(jnp.where(r == r_max, tok, S - 1))
    base = pl.multiple_of((idx // 16) * 16, 16)
    grp = x_v[pl.ds(base, 16), :].astype(f32)
    sel = lax.broadcasted_iota(jnp.int32, (16, 1), 0) == idx - base
    x_sel = jnp.sum(jnp.where(sel, grp, 0.0), axis=0, keepdims=True)
    xb_v[...] = _col_bcast(x_sel)
    z_v[...] = jnp.broadcast_to(_rnd(jnp.sum(z_v[...], axis=1, keepdims=True)), (D, 128))
    y_v[...] = jnp.zeros_like(y_v)
    g_v[...] = jnp.zeros_like(g_v)

    def mid(i, c):
        for cp in f_copies(i):
            cp.wait()
        rows = pl.ds(pl.multiple_of(i * SB, SB), SB)
        g_v[...] += jnp.dot(pt_v[1, i], x_v[rows, :], preferred_element_type=f32)

        pq = pt_v[0, i].astype(f32).reshape(H, DH, SB)
        zz = _lanes(z_v[...], SB // 128).reshape(H, DH, SB)
        den = _rnd(jnp.sum(pq * zz, axis=1, keepdims=True)) + 1e-6
        pn = (pq * (1.0 / den)).reshape(D, SB)
        pn_v[rows, :] = pn.T.astype(bf16)

        ag = jnp.zeros((8, FC), f32)
        au = jnp.zeros((8, FC), f32)
        for k in range(0, D, 16):
            xk = _lanes(xb_v[k:k + 16, :], FC // 128)
            pg = wg_v[i, k:k + 16, :].astype(f32) * xk
            pu = wu_v[i, k:k + 16, :].astype(f32) * xk
            ag += pg[:8] + pg[8:]
            au += pu[:8] + pu[8:]
        hg = _rnd(jnp.sum(ag, axis=0, keepdims=True))
        hu = _rnd(jnp.sum(au, axis=0, keepdims=True))
        hb = _col_bcast(_rnd(_rnd(hg * jax.nn.sigmoid(hg)) * hu))
        ay = y_v[...]
        for k in range(0, FC, 16):
            py = wd_v[i, k:k + 16, :].astype(f32) * _lanes(hb[k:k + 16, :], D // 128)
            ay += py[:8] + py[8:]
        y_v[...] = ay
        return c
    lax.fori_loop(0, NB, mid, 0)

    w_copy(2).wait()
    w_copy(3).wait()
    same_head = (lax.broadcasted_iota(jnp.int32, (128, 128), 0) // DH
                 == lax.broadcasted_iota(jnp.int32, (128, 128), 1) // DH)
    for j in range(0, D, 128):
        kv = jnp.dot(g_v[j:j + 128, :].astype(bf16), w_v[2, :, j:j + 128],
                     preferred_element_type=f32)
        kv = jnp.where(same_head, kv, 0.0).astype(bf16)
        m_v[j:j + 128, :] = jnp.dot(kv, wo_v[j:j + 128, :],
                                    preferred_element_type=f32).astype(bf16)
    y = _rnd(_rnd(jnp.sum(y_v[...], axis=0, keepdims=True)) * _rnd(jax.nn.sigmoid(r_max)))

    def fin(i, c):
        rows = pl.ds(pl.multiple_of(i * SB, SB), SB)
        a = jnp.dot(pn_v[rows, :], m_v[...], preferred_element_type=f32)
        gate = jax.nn.sigmoid(gr_v[0, rows, :])
        xb = x_v[rows, :].astype(f32)
        hit = lax.broadcasted_iota(jnp.int32, (SB, 1), 0) == idx - i * SB
        b = xb + (xb * 0.0 + jnp.where(hit, y, 0.0))
        o_v[rows, :] = (gate * a + (1.0 - gate) * b).astype(bf16)
        o_copy(i).start()
        return c
    lax.fori_loop(0, NB, fin, 0)
    for i in range(NB):
        o_copy(i).wait()


@jax.jit
def pallas_gated_mix__linear_attn_block__moe_arch_mod__prompt_kernel(
    A_x: jax.Array,
    A_wqkv: jax.Array,
    A_wo: jax.Array,
    B_x: jax.Array,
    B_w_r: jax.Array,
    B_w_gate: jax.Array,
    B_w_up: jax.Array,
    B_w_down: jax.Array,
    gate_w: jax.Array,
):
    vec = jnp.stack([gate_w, B_w_r]).astype(f32)
    hbm = pl.BlockSpec(memory_space=pl.ANY)
    out = pl.pallas_call(
        _kernel,
        in_specs=[hbm] * 6 + [pl.BlockSpec(memory_space=pltpu.VMEM)],
        out_specs=hbm,
        out_shape=jax.ShapeDtypeStruct((S, D), bf16),
        scratch_shapes=[
            pltpu.VMEM((S, D), bf16),
            pltpu.VMEM((3, D, D), bf16),
            pltpu.VMEM((2, D, D), bf16),
            pltpu.VMEM((D, D), bf16),
            pltpu.VMEM((NB, D, FC), bf16),
            pltpu.VMEM((NB, D, FC), bf16),
            pltpu.VMEM((NB, FC, D), bf16),
            pltpu.VMEM((2, NB, D, SB), bf16),
            pltpu.VMEM((S, D), bf16),
            pltpu.VMEM((D, D), f32),
            pltpu.VMEM((D, D), bf16),
            pltpu.VMEM((2, S, 1), f32),
            pltpu.VMEM((D, 128), f32),
            pltpu.VMEM((D, 128), f32),
            pltpu.VMEM((8, D), f32),
            pltpu.VMEM((S, D), bf16),
            pltpu.SemaphoreType.DMA((NB,)),
            pltpu.SemaphoreType.DMA((4,)),
            pltpu.SemaphoreType.DMA((3, NB)),
            pltpu.SemaphoreType.DMA((NB,)),
        ],
        compiler_params=pltpu.CompilerParams(vmem_limit_bytes=110 * 1024 * 1024),
    )(A_x.reshape(S, D), A_wqkv, A_wo, B_w_gate, B_w_up, B_w_down, vec)
    return out.reshape(1, S, D)
```

```python
import jax
import jax.numpy as jnp
from jax import lax
import jax.experimental.pallas as pl
import jax.experimental.pallas.tpu as pltpu

S, D, F, H = 2048, 1024, 3584, 32
DH = D // H
T = 128
XC = 256
FC = 512
NF = F // FC
KG = 512
f32, bf16 = jnp.float32, jnp.bfloat16
NT = (((1,), (1,)), ((), ()))


def _phi(t):
    return jnp.where(t > 0, t + 1.0, jnp.exp(t)) + 1e-6


def _rnd(t):
    return t.astype(bf16).astype(f32)


def _col_bcast(row):
    n = row.shape[1]
    return jnp.concatenate(
        [jnp.broadcast_to(row[:, j:j + T], (T, T)).T for j in range(0, n, T)], axis=0)


def _lanes(t, n):
    return jnp.concatenate([t] * n, axis=1)
import functools
u32 = jnp.uint32
GK = 512
GATE = 3
STORE_AT = [768, 1536, 1792]
K_SPLIT = 768
N_SPLIT = 1792
LAST_SPLIT = 512
SR = 16
FR = 16
UP_EARLY = 3
MQ = 256
MG = 256
MF = 256
FLAGS = None


def _ld(ref, r0, n, c0, m):
    return pltpu.bitcast(ref[r0 // 2:(r0 + n) // 2, c0:c0 + m], bf16)


def _st(ref, r0, c0, val):
    n, m = val.shape
    ref[r0 // 2:(r0 + n) // 2, c0:c0 + m] = pltpu.bitcast(val.astype(bf16), jnp.uint32)


def _kernel(x_hbm, wqkv_hbm, wo_hbm, wg_hbm, wu_hbm, wd_hbm, vec_ref, out_hbm,
            x_v, w_v, wt_v, wo_v, wg_v, wu_v, wd_v, pt_v, pn_v, kv_v, gb_v, y_v, m_v, gate_v, r_v,
            z_v, xb_v, hb_v, o_v, sem_i, sem_o):
    def rows_in(i, r0, r1):
        return pltpu.make_async_copy(x_hbm.at[r0:r1], x_v.at[r0:r1], sem_i.at[i])

    def cols_in(i, c0, c1):
        return pltpu.make_async_copy(wqkv_hbm.at[:, c0:c1], w_v.at[:, c0:c1], sem_i.at[i])

    wq0, x0, wq1, x1 = cols_in(0, 0, XC), rows_in(1, 0, XC), cols_in(2, XC, 2 * XC), rows_in(3, XC, 2 * XC)
    wq2, x2, x3, wk = cols_in(4, 2 * XC, D), rows_in(5, 2 * XC, D), rows_in(6, D, S), cols_in(7, D, 2 * D)
    wg = pltpu.make_async_copy(wg_hbm, wg_v, sem_i.at[8])
    wu = pltpu.make_async_copy(wu_hbm, wu_v, sem_i.at[9])
    wv = cols_in(10, 2 * D, 3 * D)
    wo = pltpu.make_async_copy(wo_hbm, wo_v, sem_i.at[11])
    wd = pltpu.make_async_copy(wd_hbm, wd_v, sem_i.at[12])
    stores = []

    def start_store(s0, n, c0, c1):
        blk = (pl.ds(s0, n), pl.ds(c0, c1 - c0))
        stores.append(pltpu.make_async_copy(o_v.at[blk], out_hbm.at[blk], sem_o.at[len(stores)]))
        stores[-1].start()

    st = {"due": [], "go": []}
    zero = pltpu.bitcast(vec_ref[8:16, 0:T], u32)

    def due(val):
        bits = pltpu.bitcast(val, u32)
        st["due"] += [bits[r:r + 8, c:c + T] for r in range(0, bits.shape[0], 8)
                      for c in range(0, bits.shape[1], T)]

    def started(acc):
        st["go"].append(pltpu.bitcast(acc[0:8, 0:T], u32) & zero)

    def gated(val):
        if not GATE or len(st["go"]) < GATE:
            return val
        bits = pltpu.bitcast(val, u32)
        go = jnp.tile(st["go"][-GATE], (bits.shape[0] // 8, bits.shape[1] // T))
        return pltpu.bitcast(bits | go, val.dtype)

    def paced(rhs):
        if not st["due"]:
            return rhs
        tok = functools.reduce(jnp.bitwise_or, st["due"]) & zero
        st["due"] = []
        bits = pltpu.bitcast(rhs, u32)
        top = bits[0:8, 0:T] | tok
        if bits.shape[1] > T:
            top = jnp.concatenate([top, bits[0:8, T:]], axis=1)
        return pltpu.bitcast(jnp.concatenate([top, bits[8:]], axis=0), bf16)

    def transpose_w(t, c0, k0):
        wt = gated(w_v[k0:k0 + XC, t * D + c0:t * D + c0 + T]).T
        _st(wt_v.at[t], c0, k0, wt)
        due(wt)

    def scores(s0):
        xs = gated(x_v[s0:s0 + SR, :]).astype(f32)
        gl = jnp.sum(xs * vec_ref[0:1, :], axis=1, keepdims=True)
        gate = jax.nn.sigmoid(jnp.broadcast_to(gl, (SR, T)))
        gate_v[s0:s0 + SR, :] = gate
        r = jnp.sum(xs * vec_ref[1:2, :], axis=1, keepdims=True)
        r = _rnd(jnp.broadcast_to(r, (SR, T)))
        r_v[s0:s0 + SR, :] = r
        due(gate)
        due(r)

    def route_max(s0, n):
        m = jnp.max(gated(r_v[s0:s0 + n, :]).reshape(n // 8, 8, T), axis=0)
        st["m8"] = m if s0 == 0 else jnp.maximum(st["m8"], m)
        if s0 + n == S:
            st["r_max"] = jnp.max(st["m8"], axis=0, keepdims=True)
        due(st["m8"])

    def route_arg(s0, n):
        tok = lax.broadcasted_iota(jnp.int32, (n, T), 0) + s0
        cand = jnp.where(gated(r_v[s0:s0 + n, :]) == st["r_max"], tok, S - 1)
        m = jnp.min(cand.reshape(n // 8, 8, T), axis=0)
        st["i8"] = m if s0 == 0 else jnp.minimum(st["i8"], m)
        due(st["i8"])

    def route_gather():
        idx = jnp.min(st["i8"])
        base = pl.multiple_of((idx // 16) * 16, 16)
        grp = x_v[pl.ds(base, 16), :].astype(f32)
        sel = lax.broadcasted_iota(jnp.int32, (16, 1), 0) == idx - base
        st["x_sel"] = jnp.sum(jnp.where(sel, grp, 0.0), axis=0, keepdims=True)
        st["idx"] = idx

    def route_spread(k0):
        xb = _col_bcast(st["x_sel"][:, k0:k0 + T])
        xb_v[k0:k0 + T, :] = xb
        due(xb)

    def accumulate(part, first):
        part = part if first else y_v[0] + part
        y_v[0] = part
        due(part)

    def ffn_up(c, k0, k1):
        cols = slice(c * FC, (c + 1) * FC)
        for k in range(k0, k1, 16):
            xk = _lanes(gated(xb_v[k:k + 16, :]), FC // T)
            pg = wg_v[k:k + 16, cols].astype(f32) * xk
            pu = wu_v[k:k + 16, cols].astype(f32) * xk
            pg, pu = pg[:8] + pg[8:], pu[:8] + pu[8:]
            ag, au = (pg, pu) if k == k0 else (ag + pg, au + pu)
        accumulate(jnp.concatenate([ag, au], axis=1), k0 == 0)

    def ffn_act(c):
        hg = _rnd(jnp.sum(y_v[0, :, :FC], axis=0, keepdims=True))
        hu = _rnd(jnp.sum(y_v[0, :, FC:], axis=0, keepdims=True))
        hb = _col_bcast(_rnd(_rnd(hg * jax.nn.sigmoid(hg)) * hu))
        hb_v[c * FC:(c + 1) * FC, :] = hb
        due(hb)

    def ffn_down(k0, k1):
        for k in range(k0, k1, 16):
            py = wd_v[k:k + 16, :].astype(f32) * _lanes(gated(hb_v[k:k + 16, :]), D // T)
            py = py[:8] + py[8:]
            ay = py if k == k0 else ay + py
        accumulate(ay, k0 == 0)

    def ffn_finish():
        y = _rnd(_rnd(jnp.sum(y_v[0], axis=0, keepdims=True))
                 * _lanes(_rnd(jax.nn.sigmoid(st["r_max"])), D // T))
        y_v[0] = jnp.broadcast_to(y, (8, D))

    def z_finish(n0):
        z = _rnd(jnp.sum(z_v[n0:n0 + T, :], axis=1, keepdims=True))
        z = jnp.broadcast_to(z, (T, T))
        z_v[n0:n0 + T, :] = z
        due(z)

    def normalise(s0, n0):
        pq = gated(_ld(pt_v.at[0], n0, T, s0, T)).astype(f32).reshape(T // DH, DH, T)
        zz = z_v[n0:n0 + T, :].reshape(T // DH, DH, T)
        den = _rnd(jnp.sum(pq * zz, axis=1, keepdims=True)) + 1e-6
        pn = (pq * (1.0 / den)).reshape(T, T).T.astype(bf16)
        _st(pn_v, s0, n0, pn)
        due(pn)

    def proj(t, n0, s0):
        acc = lax.dot_general(_ld(wt_v.at[t], n0, MQ, 0, D), paced(x_v[s0:s0 + T, :]), NT,
                              preferred_element_type=f32)
        started(acc)
        p = _phi(acc)
        _st(pt_v.at[t], n0, s0, p)
        if t == 1:
            z_v[n0:n0 + MQ, :] = p if s0 == 0 else z_v[n0:n0 + MQ, :] + p

    def proj_direct(n0, s0):
        acc = jnp.dot(x_v[s0:s0 + XC, :], paced(w_v[:, n0:n0 + T]), preferred_element_type=f32)
        started(acc)
        _st(pt_v.at[0], n0, s0, _phi(acc).T)

    def gram(n0, c0, s0):
        acc = jnp.dot(_ld(pt_v.at[1], n0, MG, s0, GK), paced(x_v[s0:s0 + GK, c0:c0 + T]),
                      preferred_element_type=f32)
        started(acc)
        st["g"] = acc if s0 == 0 else st["g"] + acc
        if s0 + GK == S:
            _st(gb_v, n0, c0, st["g"])

    def kv_block(n0):
        kv = jnp.dot(_ld(gb_v, n0, T, 0, D), w_v[:, 2 * D + n0:2 * D + n0 + T], preferred_element_type=f32)
        same_head = (lax.broadcasted_iota(jnp.int32, (T, T), 0) // DH
                     == lax.broadcasted_iota(jnp.int32, (T, T), 1) // DH)
        _st(kv_v, n0, 0, jnp.where(same_head, kv, 0.0))

    def m_block(n0, c0):
        _st(m_v, n0, c0, jnp.dot(_ld(kv_v, n0, T, 0, T), wo_v[n0:n0 + T, c0:c0 + 4 * T],
                                 preferred_element_type=f32))

    def final(s0, c0):
        rows, cols = slice(s0, s0 + MF), slice(c0, c0 + T)
        a = jnp.dot(_ld(pn_v, s0, MF, 0, D), paced(_ld(m_v, 0, D, c0, T)), preferred_element_type=f32)
        started(a)
        gate = gate_v[rows, :]
        xs = x_v[rows, cols].astype(f32)
        hit = lax.broadcasted_iota(jnp.int32, (MF, T), 0) == st["idx"] - s0
        y = jnp.broadcast_to(y_v[0, 0:1, cols], (MF, T))
        b = xs + (xs * 0.0 + jnp.where(hit, y, 0.0))
        o_v[rows, cols] = (gate * a + (1.0 - gate) * b).astype(bf16)
        if s0 + MF == S:
            if (c0 + T) % LAST_SPLIT == 0:
                start_store(s0, MF, c0 + T - LAST_SPLIT, c0 + T)
        elif c0 + T == D and s0 + MF in STORE_AT:
            r0 = ([0] + STORE_AT)[STORE_AT.index(s0 + MF)]
            start_store(r0, s0 + MF - r0, 0, D)

    def run(pieces, *lanes):
        n, done = len(pieces), [0] * len(lanes)
        for p, piece in enumerate(pieces):
            for fn, *args in piece:
                fn(*args)
            for li, lane in enumerate(lanes):
                upto = -(-len(lane) * (p + 1) // n)
                for fn, *args in lane[done[li]:upto]:
                    fn(*args)
                done[li] = upto
        st["due"] = []

    tiles_n = range(0, D, T)
    for cp in (wq0, x0, wq1, x1, wq2, x2, x3, wk, wg, wu, wv, wo, wd):
        cp.start()

    def proj_tiles(t, s_lo, s_hi, n_hi=D):
        return [[(proj, t, n0, s0)] for s0 in range(s_lo, s_hi, T) for n0 in range(0, n_hi, MQ)]

    def w_tiles(t, n_lo, n_hi):
        return [(transpose_w, t, n0, k0) for n0 in range(n_lo, n_hi, T) for k0 in range(0, D, XC)]

    def score_tiles(s_lo, s_hi):
        return [(scores, s0) for s0 in range(s_lo, s_hi, SR)]

    wq0.wait()
    x0.wait()
    run([[(proj_direct, n0, 0)] for n0 in (0, T)], w_tiles(0, 0, XC))
    wq1.wait()
    run([[(proj_direct, n0, 0)] for n0 in (2 * T, 3 * T)],
        w_tiles(0, XC, 2 * XC))
    x1.wait()
    run(proj_tiles(0, XC, 2 * XC, 2 * XC), score_tiles(0, XC))
    wq2.wait()
    run([[(proj_direct, n0, s0)] for n0 in range(2 * XC, D, T) for s0 in (0, XC)],
        w_tiles(0, 2 * XC, D))
    x2.wait()
    run(proj_tiles(0, 2 * XC, D), score_tiles(XC, D))
    x3.wait()
    wk.wait()
    run(proj_tiles(0, D, S - MF), w_tiles(1, 0, D), score_tiles(D, S))

    def chain(n0):
        blocks = range(n0, n0 + MG, T)
        return ([[(kv_block, n)] for n in blocks],
                [[(m_block, n, c)] for n in blocks for c in (0, 4 * T)])

    def gram_rows(n0):
        pieces = []
        for c0 in tiles_n:
            pieces += [[(gram, n0, c0, s0)] for s0 in range(0, S, GK)]
            if n0 > 0 and c0 in (T, 3 * T):
                pieces += chain(n0 - MG)[c0 // (2 * T)]
        return pieces

    route = ([(route_max, s0, 256) for s0 in range(0, S, 256)]
             + [(route_arg, s0, 128) for s0 in range(0, S, 128)] + [(route_gather,)])
    run(proj_tiles(1, 0, K_SPLIT - 2 * T), route)
    run(proj_tiles(1, K_SPLIT - 2 * T, K_SPLIT), [(route_spread, k0) for k0 in tiles_n])
    wg.wait()
    wu.wait()
    up = []
    for c in range(NF):
        up += [(ffn_up, c, k, k + FR) for k in range(0, D, FR)] + [(ffn_act, c)]
    run(proj_tiles(1, K_SPLIT, S) + gram_rows(0), up)

    wv.wait()
    wo.wait()
    wd.wait()
    last = proj_tiles(0, S - MF, S)
    kvs, ms = chain(D - MG)
    run(sum([gram_rows(n0) for n0 in range(MG, D, MG)], []) + last[:1] + kvs + last[1:2] + ms + last[2:],
        [(ffn_down, k, k + FR) for k in range(0, F, FR)] + [(ffn_finish,)],
        [(z_finish, n0) for n0 in tiles_n]
        + [(normalise, s0, n0) for s0 in range(0, N_SPLIT, T) for n0 in tiles_n])

    later = [(normalise, s0, n0) for s0 in range(N_SPLIT, S, T) for n0 in tiles_n]
    for s0 in range(0, S, MF):
        run([[(final, s0, c0)] for c0 in tiles_n], later[:MF // T * len(tiles_n)])
        later = later[MF // T * len(tiles_n):]
    for cp in stores:
        cp.wait()


@jax.jit
def pallas_gated_mix__linear_attn_block__moe_arch_mod__prompt_kernel(
    A_x: jax.Array,
    A_wqkv: jax.Array,
    A_wo: jax.Array,
    B_x: jax.Array,
    B_w_r: jax.Array,
    B_w_gate: jax.Array,
    B_w_up: jax.Array,
    B_w_down: jax.Array,
    gate_w: jax.Array,
):
    del B_x
    vec = jnp.pad(jnp.stack([gate_w, B_w_r]).astype(f32), ((0, 14), (0, 0)))
    hbm = pl.BlockSpec(memory_space=pl.ANY)
    out = pl.pallas_call(
        _kernel,
        in_specs=[hbm] * 6 + [pl.BlockSpec(memory_space=pltpu.VMEM)],
        out_specs=hbm,
        out_shape=jax.ShapeDtypeStruct((S, D), bf16),
        scratch_shapes=[
            pltpu.VMEM((S, D), bf16),
            pltpu.VMEM((D, 3 * D), bf16),
            pltpu.VMEM((2, D // 2, D), u32),
            pltpu.VMEM((D, D), bf16),
            pltpu.VMEM((D, F), bf16),
            pltpu.VMEM((D, F), bf16),
            pltpu.VMEM((F, D), bf16),
            pltpu.VMEM((2, D // 2, S), u32),
            pltpu.VMEM((S // 2, D), u32),
            pltpu.VMEM((D // 2, T), u32),
            pltpu.VMEM((D // 2, D), u32),
            pltpu.VMEM((1, 8, D), f32),
            pltpu.VMEM((D // 2, D), u32),
            pltpu.VMEM((S, T), f32),
            pltpu.VMEM((S, T), f32),
            pltpu.VMEM((D, T), f32),
            pltpu.VMEM((D, T), f32),
            pltpu.VMEM((F, T), f32),
            pltpu.VMEM((S, D), bf16),
            pltpu.SemaphoreType.DMA((13,)),
            pltpu.SemaphoreType.DMA((len(STORE_AT) + D // LAST_SPLIT,)),
        ],
        compiler_params=pltpu.CompilerParams(vmem_limit_bytes=110 * 1024 * 1024, flags=FLAGS),
    )(A_x.reshape(S, D), A_wqkv, A_wo, B_w_gate, B_w_up, B_w_down, vec)
    return out.reshape(1, S, D)
```

```python
import jax
import jax.numpy as jnp
from jax import lax
import jax.experimental.pallas as pl
import jax.experimental.pallas.tpu as pltpu

S, D, F, H = 2048, 1024, 3584, 32
DH = D // H
T = 128
XC = 256
FC = 512
NF = F // FC
KG = 512
f32, bf16 = jnp.float32, jnp.bfloat16
NT = (((1,), (1,)), ((), ()))


def _phi(t):
    return jnp.where(t > 0, t + 1.0, jnp.exp(t)) + 1e-6


def _rnd(t):
    return t.astype(bf16).astype(f32)


def _col_bcast(row):
    n = row.shape[1]
    return jnp.concatenate(
        [jnp.broadcast_to(row[:, j:j + T], (T, T)).T for j in range(0, n, T)], axis=0)


def _lanes(t, n):
    return jnp.concatenate([t] * n, axis=1)
import functools
u32 = jnp.uint32
GK = 512
GATE = 4
OR_Q = True
OR_G = True
STORE_AT = [1024, 1664, 1920]
K_SPLIT = 896
N_SPLIT = 1792
LAST_SPLIT = 512
SR = 16
FR = 16
UP_EARLY = 3
MQ = 128
MG = 128
MF = 128
FLAGS = None


def _ld(ref, r0, n, c0, m):
    return pltpu.bitcast(ref[r0 // 2:(r0 + n) // 2, c0:c0 + m], bf16)


def _st(ref, r0, c0, val):
    n, m = val.shape
    ref[r0 // 2:(r0 + n) // 2, c0:c0 + m] = pltpu.bitcast(val.astype(bf16), jnp.uint32)


def _kernel(x_hbm, wqkv_hbm, wo_hbm, wg_hbm, wu_hbm, wd_hbm, gw_ref, wr_ref, out_hbm,
            x_v, w_v, wt_v, wo_v, wg_v, wu_v, wd_v, pt_v, pn_v, kv_v, gb_v, y_v, m_v, gate_v, r_v,
            z_v, xb_v, hb_v, o_v, sem_i, sem_o):
    def rows_in(i, r0, r1):
        return pltpu.make_async_copy(x_hbm.at[r0:r1], x_v.at[r0:r1], sem_i.at[i])

    def cols_in(i, c0, c1):
        return pltpu.make_async_copy(wqkv_hbm.at[:, c0:c1], w_v.at[:, c0:c1], sem_i.at[i])

    wq0, x0, wq1, x1 = cols_in(0, 0, XC), rows_in(1, 0, XC), cols_in(2, XC, 2 * XC), rows_in(3, XC, 2 * XC)
    wq2, x2, x3, wk = cols_in(4, 2 * XC, D), rows_in(5, 2 * XC, D), rows_in(6, D, S), cols_in(7, D, 2 * D)
    wg = pltpu.make_async_copy(wg_hbm, wg_v, sem_i.at[8])
    wu = pltpu.make_async_copy(wu_hbm, wu_v, sem_i.at[9])
    wv = cols_in(10, 2 * D, 3 * D)
    wo = pltpu.make_async_copy(wo_hbm, wo_v, sem_i.at[11])
    wd = pltpu.make_async_copy(wd_hbm, wd_v, sem_i.at[12])
    stores = []

    def start_store(s0, n, c0, c1):
        blk = (pl.ds(s0, n), pl.ds(c0, c1 - c0))
        stores.append(pltpu.make_async_copy(o_v.at[blk], out_hbm.at[blk], sem_o.at[len(stores)]))
        stores[-1].start()

    st = {"due": [], "go": []}
    gate_w = gw_ref[...].astype(f32).reshape(1, D)
    w_r = wr_ref[...].astype(f32).reshape(1, D)
    bits = pltpu.bitcast(jnp.broadcast_to(gate_w[:, 0:T], (8, T)), u32)
    zero = (bits >> 31) & (~bits >> 31)

    def due(val):
        bits = pltpu.bitcast(val, u32)
        st["due"] += [bits[r:r + 8, c:c + T] for r in range(0, bits.shape[0], 8)
                      for c in range(0, bits.shape[1], T)]

    def lhs(ref, r0, n, c0, m, on):
        bits = ref[r0 // 2:(r0 + n) // 2, c0:c0 + m]
        if on:
            bits = bits | jnp.tile(zero, (n // 16, m // T))
        return pltpu.bitcast(bits, bf16)

    def started(acc):
        st["go"].append(pltpu.bitcast(acc[0:8, 0:T], u32) & zero)

    def gated(val):
        if not GATE or len(st["go"]) < GATE:
            return val
        bits = pltpu.bitcast(val, u32)
        go = jnp.tile(st["go"][-GATE], (bits.shape[0] // 8, bits.shape[1] // T))
        return pltpu.bitcast(bits | go, val.dtype)

    def paced(rhs):
        if not st["due"]:
            return rhs
        tok = functools.reduce(jnp.bitwise_or, st["due"]) & zero
        st["due"] = []
        bits = pltpu.bitcast(rhs, u32)
        top = bits[0:8, 0:T] | tok
        if bits.shape[1] > T:
            top = jnp.concatenate([top, bits[0:8, T:]], axis=1)
        return pltpu.bitcast(jnp.concatenate([top, bits[8:]], axis=0), bf16)

    def transpose_w(t, c0, k0):
        wt = gated(w_v[k0:k0 + XC, t * D + c0:t * D + c0 + T]).T
        _st(wt_v.at[t], c0, k0, wt)
        due(wt)

    def scores(s0):
        xs = gated(x_v[s0:s0 + SR, :]).astype(f32)
        gl = jnp.sum(xs * gate_w, axis=1, keepdims=True)
        gate = jax.nn.sigmoid(jnp.broadcast_to(gl, (SR, T)))
        gate_v[s0:s0 + SR, :] = gate
        r = jnp.sum(xs * w_r, axis=1, keepdims=True)
        r = _rnd(jnp.broadcast_to(r, (SR, T)))
        r_v[s0:s0 + SR, :] = r
        due(gate)
        due(r)

    def route_max(s0, n):
        m = jnp.max(gated(r_v[s0:s0 + n, :]).reshape(n // 8, 8, T), axis=0)
        st["m8"] = m if s0 == 0 else jnp.maximum(st["m8"], m)
        if s0 + n == S:
            st["r_max"] = jnp.max(st["m8"], axis=0, keepdims=True)
        due(st["m8"])

    def route_arg(s0, n):
        tok = lax.broadcasted_iota(jnp.int32, (n, T), 0) + s0
        cand = jnp.where(gated(r_v[s0:s0 + n, :]) == st["r_max"], tok, S - 1)
        m = jnp.min(cand.reshape(n // 8, 8, T), axis=0)
        st["i8"] = m if s0 == 0 else jnp.minimum(st["i8"], m)
        due(st["i8"])

    def route_gather():
        idx = jnp.min(st["i8"])
        base = pl.multiple_of((idx // 16) * 16, 16)
        grp = x_v[pl.ds(base, 16), :].astype(f32)
        sel = lax.broadcasted_iota(jnp.int32, (16, 1), 0) == idx - base
        st["x_sel"] = jnp.sum(jnp.where(sel, grp, 0.0), axis=0, keepdims=True)
        st["idx"] = idx

    def route_spread(k0):
        xb = _col_bcast(st["x_sel"][:, k0:k0 + T])
        xb_v[k0:k0 + T, :] = xb
        due(xb)

    def accumulate(part, first):
        part = part if first else y_v[0] + part
        y_v[0] = part
        due(part)

    def ffn_up(c, k0, k1):
        cols = slice(c * FC, (c + 1) * FC)
        for k in range(k0, k1, 16):
            xk = _lanes(gated(xb_v[k:k + 16, :]), FC // T)
            pg = wg_v[k:k + 16, cols].astype(f32) * xk
            pu = wu_v[k:k + 16, cols].astype(f32) * xk
            pg, pu = pg[:8] + pg[8:], pu[:8] + pu[8:]
            ag, au = (pg, pu) if k == k0 else (ag + pg, au + pu)
        accumulate(jnp.concatenate([ag, au], axis=1), k0 == 0)

    def ffn_act(c):
        hg = _rnd(jnp.sum(y_v[0, :, :FC], axis=0, keepdims=True))
        hu = _rnd(jnp.sum(y_v[0, :, FC:], axis=0, keepdims=True))
        hb = _col_bcast(_rnd(_rnd(hg * jax.nn.sigmoid(hg)) * hu))
        hb_v[c * FC:(c + 1) * FC, :] = hb
        due(hb)

    def ffn_down(k0, k1):
        for k in range(k0, k1, 16):
            py = wd_v[k:k + 16, :].astype(f32) * _lanes(gated(hb_v[k:k + 16, :]), D // T)
            py = py[:8] + py[8:]
            ay = py if k == k0 else ay + py
        accumulate(ay, k0 == 0)

    def ffn_finish():
        y = _rnd(_rnd(jnp.sum(y_v[0], axis=0, keepdims=True))
                 * _lanes(_rnd(jax.nn.sigmoid(st["r_max"])), D // T))
        y_v[0] = jnp.broadcast_to(y, (8, D))

    def z_finish(n0):
        z = _rnd(jnp.sum(z_v[n0:n0 + T, :], axis=1, keepdims=True))
        z = jnp.broadcast_to(z, (T, T))
        z_v[n0:n0 + T, :] = z
        due(z)

    def normalise(s0, n0):
        pq = gated(_ld(pt_v.at[0], n0, T, s0, T)).astype(f32).reshape(T // DH, DH, T)
        zz = z_v[n0:n0 + T, :].reshape(T // DH, DH, T)
        den = _rnd(jnp.sum(pq * zz, axis=1, keepdims=True)) + 1e-6
        pn = (pq * (1.0 / den)).reshape(T, T).T.astype(bf16)
        _st(pn_v, s0, n0, pn)
        due(pn)

    def proj(t, n0, s0):
        acc = lax.dot_general(lhs(wt_v.at[t], n0, MQ, 0, D, OR_Q), paced(x_v[s0:s0 + T, :]), NT,
                              preferred_element_type=f32)
        started(acc)
        p = _phi(acc)
        _st(pt_v.at[t], n0, s0, p)
        if t == 1:
            z_v[n0:n0 + MQ, :] = p if s0 == 0 else z_v[n0:n0 + MQ, :] + p

    def proj_direct(n0, s0):
        acc = jnp.dot(x_v[s0:s0 + XC, :], paced(w_v[:, n0:n0 + T]), preferred_element_type=f32)
        started(acc)
        _st(pt_v.at[0], n0, s0, _phi(acc).T)

    def gram(n0, c0, s0):
        acc = jnp.dot(lhs(pt_v.at[1], n0, MG, s0, GK, OR_G), paced(x_v[s0:s0 + GK, c0:c0 + T]),
                      preferred_element_type=f32)
        started(acc)
        st["g"] = acc if s0 == 0 else st["g"] + acc
        if s0 + GK == S:
            _st(gb_v, n0, c0, st["g"])

    def kv_block(n0):
        kv = jnp.dot(_ld(gb_v, n0, T, 0, D), w_v[:, 2 * D + n0:2 * D + n0 + T], preferred_element_type=f32)
        same_head = (lax.broadcasted_iota(jnp.int32, (T, T), 0) // DH
                     == lax.broadcasted_iota(jnp.int32, (T, T), 1) // DH)
        _st(kv_v, n0, 0, jnp.where(same_head, kv, 0.0))

    def m_block(n0, c0):
        _st(m_v, n0, c0, jnp.dot(_ld(kv_v, n0, T, 0, T), wo_v[n0:n0 + T, c0:c0 + 4 * T],
                                 preferred_element_type=f32))

    def final(s0, c0):
        rows, cols = slice(s0, s0 + MF), slice(c0, c0 + T)
        a = jnp.dot(_ld(pn_v, s0, MF, 0, D), paced(_ld(m_v, 0, D, c0, T)), preferred_element_type=f32)
        started(a)
        gate = gate_v[rows, :]
        xs = x_v[rows, cols].astype(f32)
        hit = lax.broadcasted_iota(jnp.int32, (MF, T), 0) == st["idx"] - s0
        y = jnp.broadcast_to(y_v[0, 0:1, cols], (MF, T))
        b = xs + (xs * 0.0 + jnp.where(hit, y, 0.0))
        o_v[rows, cols] = (gate * a + (1.0 - gate) * b).astype(bf16)
        if s0 + MF == S:
            if (c0 + T) % LAST_SPLIT == 0:
                start_store(s0, MF, c0 + T - LAST_SPLIT, c0 + T)
        elif c0 + T == D and s0 + MF in STORE_AT:
            r0 = ([0] + STORE_AT)[STORE_AT.index(s0 + MF)]
            start_store(r0, s0 + MF - r0, 0, D)

    def run(pieces, *lanes):
        n, done = len(pieces), [0] * len(lanes)
        for p, piece in enumerate(pieces):
            for fn, *args in piece:
                fn(*args)
            for li, lane in enumerate(lanes):
                upto = -(-len(lane) * (p + 1) // n)
                for fn, *args in lane[done[li]:upto]:
                    fn(*args)
                done[li] = upto
        st["due"] = []

    tiles_n = range(0, D, T)
    for cp in (wq0, x0, wq1, x1, wq2, x2, x3, wk, wg, wu, wv, wo, wd):
        cp.start()

    def proj_tiles(t, s_lo, s_hi, n_hi=D):
        return [[(proj, t, n0, s0)] for s0 in range(s_lo, s_hi, T) for n0 in range(0, n_hi, MQ)]

    def w_tiles(t, n_lo, n_hi):
        return [(transpose_w, t, n0, k0) for n0 in range(n_lo, n_hi, T) for k0 in range(0, D, XC)]

    def score_tiles(s_lo, s_hi):
        return [(scores, s0) for s0 in range(s_lo, s_hi, SR)]

    wq0.wait()
    x0.wait()
    run([[(proj_direct, n0, 0)] for n0 in (0, T)], w_tiles(0, 0, XC))
    wq1.wait()
    run([[(proj_direct, n0, 0)] for n0 in (2 * T, 3 * T)],
        w_tiles(0, XC, 2 * XC))
    x1.wait()
    run(proj_tiles(0, XC, 2 * XC, 2 * XC), score_tiles(0, XC))
    wq2.wait()
    run([[(proj_direct, n0, s0)] for n0 in range(2 * XC, D, T) for s0 in (0, XC)],
        w_tiles(0, 2 * XC, D))
    x2.wait()
    run(proj_tiles(0, 2 * XC, D), score_tiles(XC, D))
    x3.wait()
    wk.wait()
    run(proj_tiles(0, D, S - MF), w_tiles(1, 0, D), score_tiles(D, S))

    def chain(n0):
        blocks = range(n0, n0 + MG, T)
        return ([[(kv_block, n)] for n in blocks],
                [[(m_block, n, c)] for n in blocks for c in (0, 4 * T)])

    def gram_rows(n0):
        pieces = []
        for c0 in tiles_n:
            pieces += [[(gram, n0, c0, s0)] for s0 in range(0, S, GK)]
            if n0 > 0 and c0 in (T, 3 * T):
                pieces += chain(n0 - MG)[c0 // (2 * T)]
        return pieces

    route = ([(route_max, s0, 256) for s0 in range(0, S, 256)]
             + [(route_arg, s0, 128) for s0 in range(0, S, 128)] + [(route_gather,)])
    run(proj_tiles(1, 0, K_SPLIT - 2 * T), route)
    run(proj_tiles(1, K_SPLIT - 2 * T, K_SPLIT), [(route_spread, k0) for k0 in tiles_n])
    wg.wait()
    wu.wait()
    up = []
    for c in range(NF):
        up += [(ffn_up, c, k, k + FR) for k in range(0, D, FR)] + [(ffn_act, c)]
    run(proj_tiles(1, K_SPLIT, S) + gram_rows(0), up)

    wv.wait()
    wo.wait()
    wd.wait()
    last = proj_tiles(0, S - MF, S)
    kvs, ms = chain(D - MG)
    run(sum([gram_rows(n0) for n0 in range(MG, D, MG)], []) + last[:1] + kvs + last[1:2] + ms + last[2:],
        [(ffn_down, k, k + FR) for k in range(0, F, FR)] + [(ffn_finish,)],
        [(z_finish, n0) for n0 in tiles_n]
        + [(normalise, s0, n0) for s0 in range(0, N_SPLIT, T) for n0 in tiles_n])

    later = [(normalise, s0, n0) for s0 in range(N_SPLIT, S, T) for n0 in tiles_n]
    for s0 in range(0, S, MF):
        run([[(final, s0, c0)] for c0 in tiles_n], later[:MF // T * len(tiles_n)])
        later = later[MF // T * len(tiles_n):]
    for cp in stores:
        cp.wait()


@jax.jit
def pallas_gated_mix__linear_attn_block__moe_arch_mod__prompt_kernel(
    A_x: jax.Array,
    A_wqkv: jax.Array,
    A_wo: jax.Array,
    B_x: jax.Array,
    B_w_r: jax.Array,
    B_w_gate: jax.Array,
    B_w_up: jax.Array,
    B_w_down: jax.Array,
    gate_w: jax.Array,
):
    del B_x
    hbm = pl.BlockSpec(memory_space=pl.ANY)
    out = pl.pallas_call(
        _kernel,
        in_specs=[hbm] * 6 + [pl.BlockSpec(memory_space=pltpu.VMEM)] * 2,
        out_specs=hbm,
        out_shape=jax.ShapeDtypeStruct((S, D), bf16),
        scratch_shapes=[
            pltpu.VMEM((S, D), bf16),
            pltpu.VMEM((D, 3 * D), bf16),
            pltpu.VMEM((2, D // 2, D), u32),
            pltpu.VMEM((D, D), bf16),
            pltpu.VMEM((D, F), bf16),
            pltpu.VMEM((D, F), bf16),
            pltpu.VMEM((F, D), bf16),
            pltpu.VMEM((2, D // 2, S), u32),
            pltpu.VMEM((S // 2, D), u32),
            pltpu.VMEM((D // 2, T), u32),
            pltpu.VMEM((D // 2, D), u32),
            pltpu.VMEM((1, 8, D), f32),
            pltpu.VMEM((D // 2, D), u32),
            pltpu.VMEM((S, T), f32),
            pltpu.VMEM((S, T), f32),
            pltpu.VMEM((D, T), f32),
            pltpu.VMEM((D, T), f32),
            pltpu.VMEM((F, T), f32),
            pltpu.VMEM((S, D), bf16),
            pltpu.SemaphoreType.DMA((13,)),
            pltpu.SemaphoreType.DMA((len(STORE_AT) + D // LAST_SPLIT,)),
        ],
        compiler_params=pltpu.CompilerParams(vmem_limit_bytes=110 * 1024 * 1024, flags=FLAGS),
    )(A_x.reshape(S, D), A_wqkv, A_wo, B_w_gate, B_w_up, B_w_down, gate_w, B_w_r)
    return out.reshape(1, S, D)
```

```python
import jax
import jax.numpy as jnp
from jax import lax
import jax.experimental.pallas as pl
import jax.experimental.pallas.tpu as pltpu

S, D, F, H = 2048, 1024, 3584, 32
DH = D // H
T = 128
XC = 256
FC = 512
NF = F // FC
KG = 512
f32, bf16 = jnp.float32, jnp.bfloat16
NT = (((1,), (1,)), ((), ()))


def _phi(t):
    return jnp.where(t > 0, t + 1.0, jnp.exp(t)) + 1e-6


def _rnd(t):
    return t.astype(bf16).astype(f32)


def _col_bcast(row):
    n = row.shape[1]
    return jnp.concatenate(
        [jnp.broadcast_to(row[:, j:j + T], (T, T)).T for j in range(0, n, T)], axis=0)


def _lanes(t, n):
    return jnp.concatenate([t] * n, axis=1)
import functools
u32 = jnp.uint32
GK = 512
GATE = 4
G_EARLY = 1
OR_Q = True
OR_G = True
STORE_AT = [1024, 1664, 1920]
K_SPLIT = 896
N_SPLIT = 1792
LAST_SPLIT = 512
SR = 16
FR = 16
UP_EARLY = 3
MQ = 128
MG = 128
MF = 128
FLAGS = None


def _ld(ref, r0, n, c0, m):
    return pltpu.bitcast(ref[r0 // 2:(r0 + n) // 2, c0:c0 + m], bf16)


def _st(ref, r0, c0, val):
    n, m = val.shape
    ref[r0 // 2:(r0 + n) // 2, c0:c0 + m] = pltpu.bitcast(val.astype(bf16), jnp.uint32)


def _kernel(x_hbm, wqkv_hbm, wo_hbm, wg_hbm, wu_hbm, wd_hbm, gw_hbm, wr_hbm, out_hbm,
            x_v, w_v, wt_v, wo_v, wg_v, wu_v, wd_v, pt_v, pn_v, kv_v, gb_v, y_v, m_v, gate_v, r_v,
            z_v, xb_v, hb_v, o_v, gw_v, wr_v, sem_i, sem_o):
    def rows_in(i, r0, r1):
        return pltpu.make_async_copy(x_hbm.at[r0:r1], x_v.at[r0:r1], sem_i.at[i])

    def cols_in(i, c0, c1):
        return pltpu.make_async_copy(wqkv_hbm.at[:, c0:c1], w_v.at[:, c0:c1], sem_i.at[i])

    wq0, x0, wq1, x1 = cols_in(0, 0, XC), rows_in(1, 0, XC), cols_in(2, XC, 2 * XC), rows_in(3, XC, 2 * XC)
    wq2, x2, x3, wk = cols_in(4, 2 * XC, D), rows_in(5, 2 * XC, D), rows_in(6, D, S), cols_in(7, D, 2 * D)
    wg = pltpu.make_async_copy(wg_hbm, wg_v, sem_i.at[8])
    wu = pltpu.make_async_copy(wu_hbm, wu_v, sem_i.at[9])
    wv = cols_in(10, 2 * D, 3 * D)
    wo = pltpu.make_async_copy(wo_hbm, wo_v, sem_i.at[11])
    wd = pltpu.make_async_copy(wd_hbm, wd_v, sem_i.at[12])
    gw = pltpu.make_async_copy(gw_hbm, gw_v, sem_i.at[13])
    wr = pltpu.make_async_copy(wr_hbm, wr_v, sem_i.at[14])
    stores = []

    def start_store(s0, n, c0, c1):
        blk = (pl.ds(s0, n), pl.ds(c0, c1 - c0))
        stores.append(pltpu.make_async_copy(o_v.at[blk], out_hbm.at[blk], sem_o.at[len(stores)]))
        stores[-1].start()

    st = {"due": [], "go": []}

    def due(val):
        bits = pltpu.bitcast(val, u32)
        st["due"] += [bits[r:r + 8, c:c + T] for r in range(0, bits.shape[0], 8)
                      for c in range(0, bits.shape[1], T)]

    def lhs(ref, r0, n, c0, m, on):
        bits = ref[r0 // 2:(r0 + n) // 2, c0:c0 + m]
        if on:
            bits = bits | jnp.tile(zero, (n // 16, m // T))
        return pltpu.bitcast(bits, bf16)

    def started(acc):
        st["go"].append(pltpu.bitcast(acc[0:8, 0:T], u32) & zero)

    def gated(val):
        if not GATE or len(st["go"]) < GATE:
            return val
        bits = pltpu.bitcast(val, u32)
        go = jnp.tile(st["go"][-GATE], (bits.shape[0] // 8, bits.shape[1] // T))
        return pltpu.bitcast(bits | go, val.dtype)

    def paced(rhs):
        if not st["due"]:
            return rhs
        tok = functools.reduce(jnp.bitwise_or, st["due"]) & zero
        st["due"] = []
        bits = pltpu.bitcast(rhs, u32)
        top = bits[0:8, 0:T] | tok
        if bits.shape[1] > T:
            top = jnp.concatenate([top, bits[0:8, T:]], axis=1)
        return pltpu.bitcast(jnp.concatenate([top, bits[8:]], axis=0), bf16)

    def transpose_w(t, c0, k0):
        wt = gated(w_v[k0:k0 + XC, t * D + c0:t * D + c0 + T]).T
        _st(wt_v.at[t], c0, k0, wt)
        due(wt)

    def scores(s0):
        xs = gated(x_v[s0:s0 + SR, :]).astype(f32)
        gl = jnp.sum(xs * st["gate_w"], axis=1, keepdims=True)
        gate = jax.nn.sigmoid(jnp.broadcast_to(gl, (SR, T)))
        gate_v[s0:s0 + SR, :] = gate
        r = jnp.sum(xs * st["w_r"], axis=1, keepdims=True)
        r = _rnd(jnp.broadcast_to(r, (SR, T)))
        r_v[s0:s0 + SR, :] = r
        due(gate)
        due(r)

    def route_max(s0, n):
        m = jnp.max(gated(r_v[s0:s0 + n, :]).reshape(n // 8, 8, T), axis=0)
        st["m8"] = m if s0 == 0 else jnp.maximum(st["m8"], m)
        if s0 + n == S:
            st["r_max"] = jnp.max(st["m8"], axis=0, keepdims=True)
        due(st["m8"])

    def route_arg(s0, n):
        tok = lax.broadcasted_iota(jnp.int32, (n, T), 0) + s0
        cand = jnp.where(gated(r_v[s0:s0 + n, :]) == st["r_max"], tok, S - 1)
        m = jnp.min(cand.reshape(n // 8, 8, T), axis=0)
        st["i8"] = m if s0 == 0 else jnp.minimum(st["i8"], m)
        due(st["i8"])

    def route_gather():
        idx = jnp.min(st["i8"])
        base = pl.multiple_of((idx // 16) * 16, 16)
        grp = x_v[pl.ds(base, 16), :].astype(f32)
        sel = lax.broadcasted_iota(jnp.int32, (16, 1), 0) == idx - base
        st["x_sel"] = jnp.sum(jnp.where(sel, grp, 0.0), axis=0, keepdims=True)
        st["idx"] = idx

    def route_spread(k0):
        xb = _col_bcast(st["x_sel"][:, k0:k0 + T])
        xb_v[k0:k0 + T, :] = xb
        due(xb)

    def accumulate(part, first):
        part = part if first else y_v[0] + part
        y_v[0] = part
        due(part)

    def ffn_up(c, k0, k1):
        cols = slice(c * FC, (c + 1) * FC)
        for k in range(k0, k1, 16):
            xk = _lanes(gated(xb_v[k:k + 16, :]), FC // T)
            pg = wg_v[k:k + 16, cols].astype(f32) * xk
            pu = wu_v[k:k + 16, cols].astype(f32) * xk
            pg, pu = pg[:8] + pg[8:], pu[:8] + pu[8:]
            ag, au = (pg, pu) if k == k0 else (ag + pg, au + pu)
        accumulate(jnp.concatenate([ag, au], axis=1), k0 == 0)

    def ffn_act(c):
        hg = _rnd(jnp.sum(y_v[0, :, :FC], axis=0, keepdims=True))
        hu = _rnd(jnp.sum(y_v[0, :, FC:], axis=0, keepdims=True))
        hb = _col_bcast(_rnd(_rnd(hg * jax.nn.sigmoid(hg)) * hu))
        hb_v[c * FC:(c + 1) * FC, :] = hb
        due(hb)

    def ffn_down(k0, k1):
        for k in range(k0, k1, 16):
            py = wd_v[k:k + 16, :].astype(f32) * _lanes(gated(hb_v[k:k + 16, :]), D // T)
            py = py[:8] + py[8:]
            ay = py if k == k0 else ay + py
        accumulate(ay, k0 == 0)

    def ffn_finish():
        y = _rnd(_rnd(jnp.sum(y_v[0], axis=0, keepdims=True))
                 * _lanes(_rnd(jax.nn.sigmoid(st["r_max"])), D // T))
        y_v[0] = jnp.broadcast_to(y, (8, D))

    def z_finish(n0):
        z = _rnd(jnp.sum(z_v[n0:n0 + T, :], axis=1, keepdims=True))
        z = jnp.broadcast_to(z, (T, T))
        z_v[n0:n0 + T, :] = z
        due(z)

    def normalise(s0, n0):
        pq = gated(_ld(pt_v.at[0], n0, T, s0, T)).astype(f32).reshape(T // DH, DH, T)
        zz = z_v[n0:n0 + T, :].reshape(T // DH, DH, T)
        den = _rnd(jnp.sum(pq * zz, axis=1, keepdims=True)) + 1e-6
        pn = (pq * (1.0 / den)).reshape(T, T).T.astype(bf16)
        _st(pn_v, s0, n0, pn)
        due(pn)

    def proj(t, n0, s0):
        acc = lax.dot_general(lhs(wt_v.at[t], n0, MQ, 0, D, OR_Q), paced(x_v[s0:s0 + T, :]), NT,
                              preferred_element_type=f32)
        started(acc)
        p = _phi(acc)
        _st(pt_v.at[t], n0, s0, p)
        if t == 1:
            z_v[n0:n0 + MQ, :] = p if s0 == 0 else z_v[n0:n0 + MQ, :] + p

    def proj_direct(n0, s0):
        acc = jnp.dot(x_v[s0:s0 + XC, :], paced(w_v[:, n0:n0 + T]), preferred_element_type=f32)
        started(acc)
        _st(pt_v.at[0], n0, s0, _phi(acc).T)

    def gram(n0, c0, s0):
        acc = jnp.dot(lhs(pt_v.at[1], n0, MG, s0, GK, OR_G), paced(x_v[s0:s0 + GK, c0:c0 + T]),
                      preferred_element_type=f32)
        started(acc)
        st["g"] = acc if s0 == 0 else st["g"] + acc
        if s0 + GK == S:
            _st(gb_v, n0, c0, st["g"])

    def kv_block(n0):
        kv = jnp.dot(_ld(gb_v, n0, T, 0, D), w_v[:, 2 * D + n0:2 * D + n0 + T], preferred_element_type=f32)
        same_head = (lax.broadcasted_iota(jnp.int32, (T, T), 0) // DH
                     == lax.broadcasted_iota(jnp.int32, (T, T), 1) // DH)
        _st(kv_v, n0, 0, jnp.where(same_head, kv, 0.0))

    def m_block(n0, c0):
        _st(m_v, n0, c0, jnp.dot(_ld(kv_v, n0, T, 0, T), wo_v[n0:n0 + T, c0:c0 + 4 * T],
                                 preferred_element_type=f32))

    def final(s0, c0):
        rows, cols = slice(s0, s0 + MF), slice(c0, c0 + T)
        a = jnp.dot(_ld(pn_v, s0, MF, 0, D), paced(_ld(m_v, 0, D, c0, T)), preferred_element_type=f32)
        started(a)
        gate = gate_v[rows, :]
        xs = x_v[rows, cols].astype(f32)
        hit = lax.broadcasted_iota(jnp.int32, (MF, T), 0) == st["idx"] - s0
        y = jnp.broadcast_to(y_v[0, 0:1, cols], (MF, T))
        b = xs + (xs * 0.0 + jnp.where(hit, y, 0.0))
        o_v[rows, cols] = (gate * a + (1.0 - gate) * b).astype(bf16)
        if s0 + MF == S:
            if (c0 + T) % LAST_SPLIT == 0:
                start_store(s0, MF, c0 + T - LAST_SPLIT, c0 + T)
        elif c0 + T == D and s0 + MF in STORE_AT:
            r0 = ([0] + STORE_AT)[STORE_AT.index(s0 + MF)]
            start_store(r0, s0 + MF - r0, 0, D)

    def run(pieces, *lanes):
        n, done = len(pieces), [0] * len(lanes)
        for p, piece in enumerate(pieces):
            for fn, *args in piece:
                fn(*args)
            for li, lane in enumerate(lanes):
                upto = -(-len(lane) * (p + 1) // n)
                for fn, *args in lane[done[li]:upto]:
                    fn(*args)
                done[li] = upto
        st["due"] = []

    tiles_n = range(0, D, T)
    for cp in (wq0, x0, wq1, gw, wr, x1, wq2, x2, x3, wk, wg, wu, wv, wo, wd):
        cp.start()

    def proj_tiles(t, s_lo, s_hi, n_hi=D):
        return [[(proj, t, n0, s0)] for s0 in range(s_lo, s_hi, T) for n0 in range(0, n_hi, MQ)]

    def w_tiles(t, n_lo, n_hi):
        return [(transpose_w, t, n0, k0) for n0 in range(n_lo, n_hi, T) for k0 in range(0, D, XC)]

    def score_tiles(s_lo, s_hi):
        return [(scores, s0) for s0 in range(s_lo, s_hi, SR)]

    wq0.wait()
    x0.wait()
    bits = pltpu.bitcast(x_v[0:16, 0:T], u32)
    zero = (bits >> 31) & (~bits >> 31)
    run([[(proj_direct, n0, 0)] for n0 in (0, T)], w_tiles(0, 0, XC))
    wq1.wait()
    run([[(proj_direct, n0, 0)] for n0 in (2 * T, 3 * T)],
        w_tiles(0, XC, 2 * XC))
    gw.wait()
    wr.wait()
    x1.wait()
    st["gate_w"] = gw_v[...].astype(f32).reshape(1, D)
    st["w_r"] = wr_v[...].astype(f32).reshape(1, D)
    run(proj_tiles(0, XC, 2 * XC, 2 * XC), score_tiles(0, XC))
    wq2.wait()
    run([[(proj_direct, n0, s0)] for n0 in range(2 * XC, D, T) for s0 in (0, XC)],
        w_tiles(0, 2 * XC, D))
    x2.wait()
    run(proj_tiles(0, 2 * XC, D), score_tiles(XC, D))
    x3.wait()
    wk.wait()
    run(proj_tiles(0, D, S - MF), w_tiles(1, 0, D), score_tiles(D, S))

    def chain(n0):
        blocks = range(n0, n0 + MG, T)
        return ([[(kv_block, n)] for n in blocks],
                [[(m_block, n, c)] for n in blocks for c in (0, 4 * T)])

    def gram_rows(n0):
        pieces = []
        for c0 in tiles_n:
            pieces += [[(gram, n0, c0, s0)] for s0 in range(0, S, GK)]
            if n0 >= G_EARLY * MG and c0 in (T, 3 * T):
                pieces += chain(n0 - MG)[c0 // (2 * T)]
            if n0 == G_EARLY * MG and c0 in (5 * T, 7 * T):
                for n1 in range(0, n0 - MG, MG):
                    pieces += chain(n1)[(c0 - 4 * T) // (2 * T)]
        return pieces

    route = ([(route_max, s0, 256) for s0 in range(0, S, 256)]
             + [(route_arg, s0, 128) for s0 in range(0, S, 128)] + [(route_gather,)])
    run(proj_tiles(1, 0, K_SPLIT - 2 * T), route)
    run(proj_tiles(1, K_SPLIT - 2 * T, K_SPLIT), [(route_spread, k0) for k0 in tiles_n])
    wg.wait()
    wu.wait()
    up = []
    for c in range(NF):
        up += [(ffn_up, c, k, k + FR) for k in range(0, D, FR)] + [(ffn_act, c)]
    run(proj_tiles(1, K_SPLIT, S) + sum([gram_rows(n0) for n0 in range(0, G_EARLY * MG, MG)], []), up)

    wv.wait()
    wo.wait()
    wd.wait()
    last = proj_tiles(0, S - MF, S)
    kvs, ms = chain(D - MG)
    run(sum([gram_rows(n0) for n0 in range(G_EARLY * MG, D, MG)], []) + last[:1] + kvs + last[1:2] + ms + last[2:],
        [(ffn_down, k, k + FR) for k in range(0, F, FR)] + [(ffn_finish,)],
        [(z_finish, n0) for n0 in tiles_n]
        + [(normalise, s0, n0) for s0 in range(0, N_SPLIT, T) for n0 in tiles_n])

    later = [(normalise, s0, n0) for s0 in range(N_SPLIT, S, T) for n0 in tiles_n]
    for s0 in range(0, S, MF):
        run([[(final, s0, c0)] for c0 in tiles_n], later[:MF // T * len(tiles_n)])
        later = later[MF // T * len(tiles_n):]
    for cp in stores:
        cp.wait()


@jax.jit
def pallas_gated_mix__linear_attn_block__moe_arch_mod__prompt_kernel(
    A_x: jax.Array,
    A_wqkv: jax.Array,
    A_wo: jax.Array,
    B_x: jax.Array,
    B_w_r: jax.Array,
    B_w_gate: jax.Array,
    B_w_up: jax.Array,
    B_w_down: jax.Array,
    gate_w: jax.Array,
):
    del B_x
    hbm = pl.BlockSpec(memory_space=pl.ANY)
    out = pl.pallas_call(
        _kernel,
        in_specs=[hbm] * 8,
        out_specs=hbm,
        out_shape=jax.ShapeDtypeStruct((S, D), bf16),
        scratch_shapes=[
            pltpu.VMEM((S, D), bf16),
            pltpu.VMEM((D, 3 * D), bf16),
            pltpu.VMEM((2, D // 2, D), u32),
            pltpu.VMEM((D, D), bf16),
            pltpu.VMEM((D, F), bf16),
            pltpu.VMEM((D, F), bf16),
            pltpu.VMEM((F, D), bf16),
            pltpu.VMEM((2, D // 2, S), u32),
            pltpu.VMEM((S // 2, D), u32),
            pltpu.VMEM((D // 2, T), u32),
            pltpu.VMEM((D // 2, D), u32),
            pltpu.VMEM((1, 8, D), f32),
            pltpu.VMEM((D // 2, D), u32),
            pltpu.VMEM((S, T), f32),
            pltpu.VMEM((S, T), f32),
            pltpu.VMEM((D, T), f32),
            pltpu.VMEM((D, T), f32),
            pltpu.VMEM((F, T), f32),
            pltpu.VMEM((S, D), bf16),
            pltpu.VMEM((D,), bf16),
            pltpu.VMEM((D,), bf16),
            pltpu.SemaphoreType.DMA((15,)),
            pltpu.SemaphoreType.DMA((len(STORE_AT) + D // LAST_SPLIT,)),
        ],
        compiler_params=pltpu.CompilerParams(vmem_limit_bytes=110 * 1024 * 1024, flags=FLAGS),
    )(A_x.reshape(S, D), A_wqkv, A_wo, B_w_gate, B_w_up, B_w_down, gate_w, B_w_r)
    return out.reshape(1, S, D)
```

```python
import functools

import jax
import jax.numpy as jnp
from jax import lax
import jax.experimental.pallas as pl
import jax.experimental.pallas.tpu as pltpu

S, D, F, H = 2048, 1024, 3584, 32
DH = D // H
T = 128
XC = 256
GK = 512
FC = 512
SR = 16
LAG = 4
K_SPLIT = 896
G_EARLY = 56
STORE_AT = (1024, 1664, S - T)
LAST_SPLIT = 512
f32, bf16, u32 = jnp.float32, jnp.bfloat16, jnp.uint32
NT = (((1,), (1,)), ((), ()))


def _phi(t):
    return jnp.where(t > 0, t + 1.0, jnp.exp(t)) + 1e-6


def _rnd(t):
    return t.astype(bf16).astype(f32)


def _lanes(t, n):
    return jnp.concatenate([t] * n, axis=1)


def _col_bcast(row):
    n = row.shape[1]
    return jnp.concatenate(
        [jnp.broadcast_to(row[:, j:j + T], (T, T)).T for j in range(0, n, T)], axis=0)


def _ld(ref, r0, n, c0, m):
    return pltpu.bitcast(ref[r0 // 2:(r0 + n) // 2, c0:c0 + m], bf16)


def _st(ref, r0, c0, val):
    n, m = val.shape
    ref[r0 // 2:(r0 + n) // 2, c0:c0 + m] = pltpu.bitcast(val.astype(bf16), u32)


def _kernel(x_hbm, wqkv_hbm, wo_hbm, wg_hbm, wu_hbm, wd_hbm, gw_hbm, wr_hbm, out_hbm,
            x_v, w_v, wt_v, wo_v, wg_v, wu_v, wd_v, pt_v, pn_v, kv_v, gb_v, y_v, m_v, gate_v, r_v,
            z_v, xb_v, hb_v, o_v, gw_v, wr_v, sem_i, sem_o):
    def rows_in(i, r0, r1):
        return pltpu.make_async_copy(x_hbm.at[r0:r1], x_v.at[r0:r1], sem_i.at[i])

    def cols_in(i, c0, c1):
        return pltpu.make_async_copy(wqkv_hbm.at[:, c0:c1], w_v.at[:, c0:c1], sem_i.at[i])

    wq0, x0 = cols_in(0, 0, XC), rows_in(1, 0, XC)
    wq1, x1 = cols_in(2, XC, 2 * XC), rows_in(3, XC, 2 * XC)
    wq2, x2 = cols_in(4, 2 * XC, D), rows_in(5, 2 * XC, D)
    x3, wk = rows_in(6, D, S), cols_in(7, D, 2 * D)
    wg = pltpu.make_async_copy(wg_hbm, wg_v, sem_i.at[8])
    wu = pltpu.make_async_copy(wu_hbm, wu_v, sem_i.at[9])
    wv = cols_in(10, 2 * D, 3 * D)
    wo = pltpu.make_async_copy(wo_hbm, wo_v, sem_i.at[11])
    wd = pltpu.make_async_copy(wd_hbm, wd_v, sem_i.at[12])
    gw = pltpu.make_async_copy(gw_hbm, gw_v, sem_i.at[13])
    wr = pltpu.make_async_copy(wr_hbm, wr_v, sem_i.at[14])
    stores = []

    def start_store(s0, n, c0, c1):
        blk = (pl.ds(s0, n), pl.ds(c0, c1 - c0))
        stores.append(pltpu.make_async_copy(o_v.at[blk], out_hbm.at[blk], sem_o.at[len(stores)]))
        stores[-1].start()

    st = {"due": [], "go": []}

    def due(val):
        bits = pltpu.bitcast(val, u32)
        st["due"] += [bits[r:r + 8, c:c + T] for r in range(0, bits.shape[0], 8)
                      for c in range(0, bits.shape[1], T)]

    def paced(rhs):
        if not st["due"]:
            return rhs
        tok = functools.reduce(jnp.bitwise_or, st["due"]) & st["zero"]
        st["due"] = []
        bits = pltpu.bitcast(rhs, u32)
        top = bits[0:8, 0:T] | tok
        return pltpu.bitcast(
            jnp.concatenate([jnp.concatenate([top, bits[0:8, T:]], axis=1)
                             if bits.shape[1] > T else top, bits[8:]], axis=0), bf16)

    def gated(val):
        if len(st["go"]) < LAG:
            return val
        bits = pltpu.bitcast(val, u32)
        go = jnp.tile(st["go"][-LAG], (bits.shape[0] // 8, bits.shape[1] // T))
        return pltpu.bitcast(bits | go, val.dtype)

    def flush():
        st.pop("tail", lambda: None)()

    def issued(acc, tail):
        flush()
        st["tail"] = tail
        st["go"].append(pltpu.bitcast(acc[0:8, 0:T], u32) & st["zero"])

    def run(pieces, *lanes):
        n, done = len(pieces), [0] * len(lanes)
        for p, (fn, *args) in enumerate(pieces):
            fn(*args)
            for li, lane in enumerate(lanes):
                upto = -(-len(lane) * (p + 1) // n)
                for side, *side_args in lane[done[li]:upto]:
                    side(*side_args)
                done[li] = upto
        st["due"] = []

    def transpose_w(t, c0, k0):
        wt = gated(w_v[k0:k0 + XC, t * D + c0:t * D + c0 + T]).T
        _st(wt_v.at[t], c0, k0, wt)
        due(wt)

    def scores(s0):
        xs = gated(x_v[s0:s0 + SR, :]).astype(f32)
        gl = jnp.sum(xs * st["gate_w"], axis=1, keepdims=True)
        gate = jax.nn.sigmoid(jnp.broadcast_to(gl, (SR, T)))
        gate_v[s0:s0 + SR, :] = gate
        r = jnp.sum(xs * st["w_r"], axis=1, keepdims=True)
        r = _rnd(jnp.broadcast_to(r, (SR, T)))
        r_v[s0:s0 + SR, :] = r
        due(gate)
        due(r)

    def route_max(s0, n):
        m = jnp.max(gated(r_v[s0:s0 + n, :]).reshape(n // 8, 8, T), axis=0)
        st["m8"] = m if s0 == 0 else jnp.maximum(st["m8"], m)
        if s0 + n == S:
            st["r_max"] = jnp.max(st["m8"], axis=0, keepdims=True)
        due(st["m8"])

    def route_arg(s0, n):
        tok = lax.broadcasted_iota(jnp.int32, (n, T), 0) + s0
        cand = jnp.where(gated(r_v[s0:s0 + n, :]) == st["r_max"], tok, S - 1)
        m = jnp.min(cand.reshape(n // 8, 8, T), axis=0)
        st["i8"] = m if s0 == 0 else jnp.minimum(st["i8"], m)
        due(st["i8"])

    def route_gather():
        idx = jnp.min(st["i8"])
        base = pl.multiple_of((idx // 16) * 16, 16)
        grp = x_v[pl.ds(base, 16), :].astype(f32)
        sel = lax.broadcasted_iota(jnp.int32, (16, 1), 0) == idx - base
        st["x_sel"] = jnp.sum(jnp.where(sel, grp, 0.0), axis=0, keepdims=True)
        st["idx"] = idx

    def route_spread(k0):
        xb = _col_bcast(st["x_sel"][:, k0:k0 + T])
        xb_v[k0:k0 + T, :] = xb
        due(xb)

    def accumulate(part, first):
        part = part if first else y_v[...] + part
        y_v[...] = part
        due(part)

    def ffn_up(c, k):
        cols = slice(c * FC, (c + 1) * FC)
        xk = _lanes(gated(xb_v[k:k + 16, :]), FC // T)
        pg = wg_v[k:k + 16, cols].astype(f32) * xk
        pu = wu_v[k:k + 16, cols].astype(f32) * xk
        pg, pu = pg[:8] + pg[8:], pu[:8] + pu[8:]
        accumulate(jnp.concatenate([pg, pu], axis=1), k == 0)

    def ffn_act(c):
        hg = _rnd(jnp.sum(y_v[:, :FC], axis=0, keepdims=True))
        hu = _rnd(jnp.sum(y_v[:, FC:], axis=0, keepdims=True))
        hb = _col_bcast(_rnd(_rnd(hg * jax.nn.sigmoid(hg)) * hu))
        hb_v[c * FC:(c + 1) * FC, :] = hb
        due(hb)

    def ffn_down(k):
        py = wd_v[k:k + 16, :].astype(f32) * _lanes(gated(hb_v[k:k + 16, :]), D // T)
        accumulate(py[:8] + py[8:], k == 0)

    def ffn_finish():
        y = _rnd(_rnd(jnp.sum(y_v[...], axis=0, keepdims=True))
                 * _lanes(_rnd(jax.nn.sigmoid(st["r_max"])), D // T))
        y_v[...] = jnp.broadcast_to(y, (8, D))

    def z_finish(n0):
        z = _rnd(jnp.sum(z_v[n0:n0 + T, :], axis=1, keepdims=True))
        z = jnp.broadcast_to(z, (T, T))
        z_v[n0:n0 + T, :] = z
        due(z)

    def normalise(s0, n0):
        pq = gated(_ld(pt_v.at[0], n0, T, s0, T)).astype(f32).reshape(T // DH, DH, T)
        zz = z_v[n0:n0 + T, :].reshape(T // DH, DH, T)
        den = _rnd(jnp.sum(pq * zz, axis=1, keepdims=True)) + 1e-6
        pn = (pq * (1.0 / den)).reshape(T, T).T.astype(bf16)
        _st(pn_v, s0, n0, pn)
        due(pn)

    def proj(t, n0, s0):
        lhs = wt_v[t, n0 // 2:(n0 + T) // 2, :] | jnp.tile(st["zero"], (T // 16, D // T))
        acc = lax.dot_general(pltpu.bitcast(lhs, bf16), paced(x_v[s0:s0 + T, :]), NT,
                              preferred_element_type=f32)

        def tail():
            p = _phi(acc)
            _st(pt_v.at[t], n0, s0, p)
            if t == 1:
                z_v[n0:n0 + T, :] = p if s0 == 0 else z_v[n0:n0 + T, :] + p
        issued(acc, tail)

    def proj_direct(n0, s0):
        acc = jnp.dot(x_v[s0:s0 + XC, :], paced(w_v[:, n0:n0 + T]), preferred_element_type=f32)
        issued(acc, lambda: _st(pt_v.at[0], n0, s0, _phi(acc).T))

    def gram(n0, c0, s0):
        acc = jnp.dot(_ld(pt_v.at[1], n0, T, s0, GK), paced(x_v[s0:s0 + GK, c0:c0 + T]),
                      preferred_element_type=f32)

        def tail():
            st["g"] = acc if s0 == 0 else st["g"] + acc
            if s0 + GK == S:
                _st(gb_v, n0, c0, st["g"])
        issued(acc, tail)

    def kv_block(n0):
        kv = jnp.dot(_ld(gb_v, n0, T, 0, D), w_v[:, 2 * D + n0:2 * D + n0 + T],
                     preferred_element_type=f32)
        same_head = (lax.broadcasted_iota(jnp.int32, (T, T), 0) // DH
                     == lax.broadcasted_iota(jnp.int32, (T, T), 1) // DH)
        _st(kv_v, n0, 0, jnp.where(same_head, kv, 0.0))

    def m_block(n0, c0):
        _st(m_v, n0, c0, jnp.dot(_ld(kv_v, n0, T, 0, T), wo_v[n0:n0 + T, c0:c0 + 4 * T],
                                 preferred_element_type=f32))

    def final(s0, c0):
        a = jnp.dot(_ld(pn_v, s0, T, 0, D), paced(_ld(m_v, 0, D, c0, T)),
                    preferred_element_type=f32)

        def tail():
            rows, cols = slice(s0, s0 + T), slice(c0, c0 + T)
            gate = gate_v[rows, :]
            xs = x_v[rows, cols].astype(f32)
            hit = lax.broadcasted_iota(jnp.int32, (T, T), 0) == st["idx"] - s0
            y = jnp.broadcast_to(y_v[0:1, cols], (T, T))
            b = xs + (xs * 0.0 + jnp.where(hit, y, 0.0))
            o_v[rows, cols] = (gate * a + (1.0 - gate) * b).astype(bf16)
            if s0 + T == S:
                if (c0 + T) % LAST_SPLIT == 0:
                    start_store(s0, T, c0 + T - LAST_SPLIT, c0 + T)
            elif c0 + T == D and s0 + T in STORE_AT:
                r0 = ((0,) + STORE_AT)[STORE_AT.index(s0 + T)]
                start_store(r0, s0 + T - r0, 0, D)
        issued(a, tail)

    tiles_n = range(0, D, T)

    def proj_tiles(t, s_lo, s_hi, n_hi=D):
        return [(proj, t, n0, s0) for s0 in range(s_lo, s_hi, T) for n0 in range(0, n_hi, T)]

    def w_tiles(t, n_lo, n_hi):
        return [(transpose_w, t, n0, k0) for n0 in range(n_lo, n_hi, T) for k0 in range(0, D, XC)]

    def score_tiles(s_lo, s_hi):
        return [(scores, s0) for s0 in range(s_lo, s_hi, SR)]

    def norm_tiles(s_lo, s_hi):
        return [(normalise, s0, n0) for s0 in range(s_lo, s_hi, T) for n0 in tiles_n]

    def m_blocks(n0):
        return [(m_block, n0, c0) for c0 in (0, 4 * T)]

    for cp in (wq0, x0, wq1, gw, wr, x1, wq2, x2, x3, wk, wg, wu, wv, wo, wd):
        cp.start()

    wq0.wait()
    x0.wait()
    bits = pltpu.bitcast(x_v[0:16, 0:T], u32)
    st["zero"] = (bits >> 31) & (~bits >> 31)
    run([(proj_direct, n0, 0) for n0 in (0, T)], w_tiles(0, 0, XC))
    wq1.wait()
    run([(proj_direct, n0, 0) for n0 in (2 * T, 3 * T)], w_tiles(0, XC, 2 * XC))
    gw.wait()
    wr.wait()
    x1.wait()
    st["gate_w"] = gw_v[...].astype(f32).reshape(1, D)
    st["w_r"] = wr_v[...].astype(f32).reshape(1, D)
    run(proj_tiles(0, XC, 2 * XC, 2 * XC), score_tiles(0, XC))
    wq2.wait()
    run([(proj_direct, n0, s0) for n0 in range(2 * XC, D, T) for s0 in (0, XC)],
        w_tiles(0, 2 * XC, D))
    x2.wait()
    run(proj_tiles(0, 2 * XC, D), score_tiles(XC, D))
    x3.wait()
    wk.wait()
    run(proj_tiles(0, D, S - T), w_tiles(1, 0, D), score_tiles(D, S))

    run(proj_tiles(1, 0, K_SPLIT - 2 * T),
        [(route_max, s0, 2 * T) for s0 in range(0, S, 2 * T)]
        + [(route_arg, s0, T) for s0 in range(0, S, T)] + [(route_gather,)])
    run(proj_tiles(1, K_SPLIT - 2 * T, K_SPLIT), [(route_spread, k0) for k0 in tiles_n])
    wg.wait()
    wu.wait()
    up, grams = [], []
    for c in range(F // FC):
        up += [(ffn_up, c, k) for k in range(0, D, 16)] + [(ffn_act, c)]
    for n0 in tiles_n:
        for c0 in tiles_n:
            grams += [(gram, n0, c0, s0) for s0 in range(0, S, GK)]
            if n0 > 0 and c0 == 5 * T:
                grams.append((kv_block, n0 - T))
            if n0 > 0 and c0 == 7 * T:
                grams += m_blocks(n0 - T)
    run(proj_tiles(1, K_SPLIT, S) + grams[:G_EARLY], up)

    wv.wait()
    wo.wait()
    wd.wait()
    last = proj_tiles(0, S - T, S)
    run(grams[G_EARLY:] + last[:1] + [(kv_block, D - T)] + last[1:2] + m_blocks(D - T) + last[2:],
        [(ffn_down, k) for k in range(0, F, 16)] + [(ffn_finish,)],
        [(z_finish, n0) for n0 in tiles_n] + norm_tiles(0, S - 2 * T))

    for s0 in range(0, S, T):
        ahead = S - 2 * T + s0
        run([(final, s0, c0) for c0 in tiles_n], norm_tiles(ahead, min(ahead + T, S)))
    flush()
    for cp in stores:
        cp.wait()


@jax.jit
def pallas_gated_mix__linear_attn_block__moe_arch_mod__prompt_kernel(
    A_x: jax.Array,
    A_wqkv: jax.Array,
    A_wo: jax.Array,
    B_x: jax.Array,
    B_w_r: jax.Array,
    B_w_gate: jax.Array,
    B_w_up: jax.Array,
    B_w_down: jax.Array,
    gate_w: jax.Array,
):
    del B_x
    hbm = pl.BlockSpec(memory_space=pl.ANY)
    out = pl.pallas_call(
        _kernel,
        in_specs=[hbm] * 8,
        out_specs=hbm,
        out_shape=jax.ShapeDtypeStruct((S, D), bf16),
        scratch_shapes=[
            pltpu.VMEM((S, D), bf16),
            pltpu.VMEM((D, 3 * D), bf16),
            pltpu.VMEM((2, D // 2, D), u32),
            pltpu.VMEM((D, D), bf16),
            pltpu.VMEM((D, F), bf16),
            pltpu.VMEM((D, F), bf16),
            pltpu.VMEM((F, D), bf16),
            pltpu.VMEM((2, D // 2, S), u32),
            pltpu.VMEM((S // 2, D), u32),
            pltpu.VMEM((D // 2, T), u32),
            pltpu.VMEM((D // 2, D), u32),
            pltpu.VMEM((8, D), f32),
            pltpu.VMEM((D // 2, D), u32),
            pltpu.VMEM((S, T), f32),
            pltpu.VMEM((S, T), f32),
            pltpu.VMEM((D, T), f32),
            pltpu.VMEM((D, T), f32),
            pltpu.VMEM((F, T), f32),
            pltpu.VMEM((S, D), bf16),
            pltpu.VMEM((D,), bf16),
            pltpu.VMEM((D,), bf16),
            pltpu.SemaphoreType.DMA((15,)),
            pltpu.SemaphoreType.DMA((len(STORE_AT) + D // LAST_SPLIT,)),
        ],
        compiler_params=pltpu.CompilerParams(vmem_limit_bytes=110 * 1024 * 1024),
    )(A_x.reshape(S, D), A_wqkv, A_wo, B_w_gate, B_w_up, B_w_down, gate_w, B_w_r)
    return out.reshape(1, S, D)
```

```python
import functools

import jax
import jax.numpy as jnp
from jax import lax
import jax.experimental.pallas as pl
import jax.experimental.pallas.tpu as pltpu

S, D, F, H = 2048, 1024, 3584, 32
DH = D // H
T = 128
XC = 256
GK = 512
FC = 512
SR = 16
LAG_N = 12
LAG_S = 4
LAG_T = 4
NBT = True
NS = 1792
RD = False
ACT = 512
LAG_D = 3
LAG_U = 4
LAG = 4
K_SPLIT = 896
G_EARLY = 56
STORE_AT = (1024, 1664, S - T)
LAST_SPLIT = 256
f32, bf16, u32 = jnp.float32, jnp.bfloat16, jnp.uint32
NT = (((1,), (1,)), ((), ()))


def _phi(t):
    return jnp.where(t > 0, t + 1.0, jnp.exp(t)) + 1e-6


def _rnd(t):
    return t.astype(bf16).astype(f32)


def _lanes(t, n):
    return jnp.concatenate([t] * n, axis=1)


def _col_bcast(row):
    n = row.shape[1]
    return jnp.concatenate(
        [jnp.broadcast_to(row[:, j:j + T], (T, T)).T for j in range(0, n, T)], axis=0)


def _ld(ref, r0, n, c0, m):
    return pltpu.bitcast(ref[r0 // 2:(r0 + n) // 2, c0:c0 + m], bf16)


def _st(ref, r0, c0, val):
    n, m = val.shape
    ref[r0 // 2:(r0 + n) // 2, c0:c0 + m] = pltpu.bitcast(val.astype(bf16), u32)


def _kernel(x_hbm, wqkv_hbm, wo_hbm, wg_hbm, wu_hbm, wd_hbm, gw_hbm, wr_hbm, out_hbm,
            x_v, w_v, wt_v, wo_v, wg_v, wu_v, wd_v, pt_v, pn_v, kv_v, gb_v, y_v, m_v, gate_v, r_v,
            z_v, xb_v, hb_v, o_v, gw_v, wr_v, sem_i, sem_o):
    def rows_in(i, r0, r1):
        return pltpu.make_async_copy(x_hbm.at[r0:r1], x_v.at[r0:r1], sem_i.at[i])

    def cols_in(i, c0, c1):
        return pltpu.make_async_copy(wqkv_hbm.at[:, c0:c1], w_v.at[:, c0:c1], sem_i.at[i])

    wq0, x0 = cols_in(0, 0, XC), rows_in(1, 0, XC)
    wq1, x1 = cols_in(2, XC, 2 * XC), rows_in(3, XC, 2 * XC)
    wq2, x2 = cols_in(4, 2 * XC, D), rows_in(5, 2 * XC, D)
    x3, wk = rows_in(6, D, S), cols_in(7, D, 2 * D)
    wg = pltpu.make_async_copy(wg_hbm, wg_v, sem_i.at[8])
    wu = pltpu.make_async_copy(wu_hbm, wu_v, sem_i.at[9])
    wv = cols_in(10, 2 * D, 3 * D)
    wo = pltpu.make_async_copy(wo_hbm, wo_v, sem_i.at[11])
    wd = pltpu.make_async_copy(wd_hbm, wd_v, sem_i.at[12])
    gw = pltpu.make_async_copy(gw_hbm, gw_v, sem_i.at[13])
    wr = pltpu.make_async_copy(wr_hbm, wr_v, sem_i.at[14])
    stores = []

    def start_store(s0, n, c0, c1):
        blk = (pl.ds(s0, n), pl.ds(c0, c1 - c0))
        stores.append(pltpu.make_async_copy(o_v.at[blk], out_hbm.at[blk], sem_o.at[len(stores)]))
        stores[-1].start()

    st = {"due": [], "go": []}

    def due(val):
        bits = pltpu.bitcast(val, u32)
        st["due"] += [bits[r:r + 8, c:c + T] for r in range(0, bits.shape[0], 8)
                      for c in range(0, bits.shape[1], T)]

    def paced(rhs):
        if not st["due"]:
            return rhs
        tok = functools.reduce(jnp.bitwise_or, st["due"]) & st["zero"]
        st["due"] = []
        bits = pltpu.bitcast(rhs, u32)
        top = bits[0:8, 0:T] | tok
        return pltpu.bitcast(
            jnp.concatenate([jnp.concatenate([top, bits[0:8, T:]], axis=1)
                             if bits.shape[1] > T else top, bits[8:]], axis=0), bf16)

    def gated(val, lag=LAG):
        if len(st["go"]) < lag:
            return val
        bits = pltpu.bitcast(val, u32)
        go = jnp.tile(st["go"][-lag], (bits.shape[0] // 8, bits.shape[1] // T))
        return pltpu.bitcast(bits | go, val.dtype)

    def flush():
        st.pop("tail", lambda: None)()

    def issued(acc, tail):
        flush()
        st["tail"] = tail
        st["go"].append(pltpu.bitcast(acc[0:8, 0:T], u32) & st["zero"])

    def run(pieces, *lanes):
        n, done = len(pieces), [0] * len(lanes)
        for p, (fn, *args) in enumerate(pieces):
            fn(*args)
            for li, lane in enumerate(lanes):
                upto = -(-len(lane) * (p + 1) // n)
                for side, *side_args in lane[done[li]:upto]:
                    side(*side_args)
                done[li] = upto
        st["due"] = []

    def transpose_w(t, c0, k0):
        wt = gated(w_v[k0:k0 + XC, t * D + c0:t * D + c0 + T], LAG_T).T
        _st(wt_v.at[t], c0, k0, wt)
        due(wt)

    def scores(s0):
        xs = gated(x_v[s0:s0 + SR, :], LAG_S).astype(f32)
        gl = jnp.sum(xs * st["gate_w"], axis=1, keepdims=True)
        gate = jax.nn.sigmoid(jnp.broadcast_to(gl, (SR, T)))
        gate_v[s0:s0 + SR, :] = gate
        r = jnp.sum(xs * st["w_r"], axis=1, keepdims=True)
        r = _rnd(jnp.broadcast_to(r, (SR, T)))
        r_v[s0:s0 + SR, :] = r
        due(gate)
        due(r)

    def route_max(s0, n):
        m = jnp.max(gated(r_v[s0:s0 + n, :]).reshape(n // 8, 8, T), axis=0)
        st["m8"] = m if s0 == 0 else jnp.maximum(st["m8"], m)
        if s0 + n == S:
            st["r_max"] = jnp.max(st["m8"], axis=0, keepdims=True)
        due(st["m8"])

    def route_arg(s0, n):
        tok = lax.broadcasted_iota(jnp.int32, (n, T), 0) + s0
        cand = jnp.where(gated(r_v[s0:s0 + n, :]) == st["r_max"], tok, S - 1)
        m = jnp.min(cand.reshape(n // 8, 8, T), axis=0)
        st["i8"] = m if s0 == 0 else jnp.minimum(st["i8"], m)
        due(st["i8"])

    def route_gather():
        idx = jnp.min(st["i8"])
        base = pl.multiple_of((idx // 16) * 16, 16)
        grp = x_v[pl.ds(base, 16), :].astype(f32)
        sel = lax.broadcasted_iota(jnp.int32, (16, 1), 0) == idx - base
        st["x_sel"] = jnp.sum(jnp.where(sel, grp, 0.0), axis=0, keepdims=True)
        st["idx"] = idx

    def route_spread(k0):
        xb = _col_bcast(st["x_sel"][:, k0:k0 + T])
        xb_v[k0:k0 + T, :] = xb
        due(xb)

    def accumulate(part, first):
        part = part if first else y_v[...] + part
        y_v[...] = part
        due(part)

    def ffn_up(c, k):
        cols = slice(c * FC, (c + 1) * FC)
        xk = _lanes(gated(xb_v[k:k + 16, :], LAG_U), FC // T)
        pg = wg_v[k:k + 16, cols].astype(f32) * xk
        pu = wu_v[k:k + 16, cols].astype(f32) * xk
        pg, pu = pg[:8] + pg[8:], pu[:8] + pu[8:]
        accumulate(jnp.concatenate([pg, pu], axis=1), k == 0)

    def ffn_act():
        hg = _rnd(jnp.sum(y_v[:, :FC], axis=0, keepdims=True))
        hu = _rnd(jnp.sum(y_v[:, FC:], axis=0, keepdims=True))
        st["h"] = _rnd(_rnd(hg * jax.nn.sigmoid(hg)) * hu)

    def ffn_spread(c, j):
        hb = _col_bcast(st["h"][:, j:j + ACT])
        hb_v[c * FC + j:c * FC + j + ACT, :] = hb
        due(hb)

    def ffn_down(k):
        py = wd_v[k:k + 16, :].astype(f32) * _lanes(gated(hb_v[k:k + 16, :], LAG_D), D // T)
        accumulate(py[:8] + py[8:], k == 0)

    def ffn_finish():
        y = _rnd(_rnd(jnp.sum(y_v[...], axis=0, keepdims=True))
                 * _lanes(_rnd(jax.nn.sigmoid(st["r_max"])), D // T))
        y_v[...] = jnp.broadcast_to(y, (8, D))

    def z_finish(n0):
        z = _rnd(jnp.sum(z_v[n0:n0 + T, :], axis=1, keepdims=True))
        z = jnp.broadcast_to(z, (T, T))
        z_v[n0:n0 + T, :] = z
        due(z)

    def normalise(s0, n0):
        pq = gated(_ld(pt_v.at[0], n0, T, s0, T), LAG_N).astype(f32).reshape(T // DH, DH, T)
        zz = z_v[n0:n0 + T, :].reshape(T // DH, DH, T)
        den = jnp.sum(pq * zz, axis=1, keepdims=True)
        den = (_rnd(den) if RD else den) + 1e-6
        pn = (pq * (1.0 / den)).reshape(T, T)
        pn = pn.astype(bf16).T if NBT else pn.T.astype(bf16)
        _st(pn_v, s0, n0, pn)
        due(pn)

    def proj(t, n0, s0):
        lhs = wt_v[t, n0 // 2:(n0 + T) // 2, :] | jnp.tile(st["zero"], (T // 16, D // T))
        acc = lax.dot_general(pltpu.bitcast(lhs, bf16), paced(x_v[s0:s0 + T, :]), NT,
                              preferred_element_type=f32)

        def tail():
            p = _phi(acc)
            _st(pt_v.at[t], n0, s0, p)
            if t == 1:
                z_v[n0:n0 + T, :] = p if s0 == 0 else z_v[n0:n0 + T, :] + p
        issued(acc, tail)

    def proj_direct(n0, s0):
        acc = jnp.dot(x_v[s0:s0 + XC, :], paced(w_v[:, n0:n0 + T]), preferred_element_type=f32)
        issued(acc, lambda: _st(pt_v.at[0], n0, s0, _phi(acc).T))

    def gram(n0, c0, s0):
        acc = jnp.dot(_ld(pt_v.at[1], n0, T, s0, GK), paced(x_v[s0:s0 + GK, c0:c0 + T]),
                      preferred_element_type=f32)

        def tail():
            st["g"] = acc if s0 == 0 else st["g"] + acc
            if s0 + GK == S:
                _st(gb_v, n0, c0, st["g"])
        issued(acc, tail)

    def kv_block(n0):
        kv = jnp.dot(_ld(gb_v, n0, T, 0, D), w_v[:, 2 * D + n0:2 * D + n0 + T],
                     preferred_element_type=f32)
        same_head = (lax.broadcasted_iota(jnp.int32, (T, T), 0) // DH
                     == lax.broadcasted_iota(jnp.int32, (T, T), 1) // DH)
        _st(kv_v, n0, 0, jnp.where(same_head, kv, 0.0))

    def m_block(n0, c0):
        _st(m_v, n0, c0, jnp.dot(_ld(kv_v, n0, T, 0, T), wo_v[n0:n0 + T, c0:c0 + 4 * T],
                                 preferred_element_type=f32))

    def final(s0, c0):
        a = jnp.dot(_ld(pn_v, s0, T, 0, D), paced(_ld(m_v, 0, D, c0, T)),
                    preferred_element_type=f32)

        def tail():
            rows, cols = slice(s0, s0 + T), slice(c0, c0 + T)
            gate = gate_v[rows, :]
            xs = x_v[rows, cols].astype(f32)
            hit = lax.broadcasted_iota(jnp.int32, (T, T), 0) == st["idx"] - s0
            y = jnp.broadcast_to(y_v[0:1, cols], (T, T))
            b = xs + (xs * 0.0 + jnp.where(hit, y, 0.0))
            o_v[rows, cols] = (gate * a + (1.0 - gate) * b).astype(bf16)
            if s0 + T == S:
                if (c0 + T) % LAST_SPLIT == 0:
                    start_store(s0, T, c0 + T - LAST_SPLIT, c0 + T)
            elif c0 + T == D and s0 + T in STORE_AT:
                r0 = ((0,) + STORE_AT)[STORE_AT.index(s0 + T)]
                start_store(r0, s0 + T - r0, 0, D)
        issued(a, tail)

    tiles_n = range(0, D, T)

    def proj_tiles(t, s_lo, s_hi, n_hi=D):
        return [(proj, t, n0, s0) for s0 in range(s_lo, s_hi, T) for n0 in range(0, n_hi, T)]

    def w_tiles(t, n_lo, n_hi):
        return [(transpose_w, t, n0, k0) for n0 in range(n_lo, n_hi, T) for k0 in range(0, D, XC)]

    def score_tiles(s_lo, s_hi):
        return [(scores, s0) for s0 in range(s_lo, s_hi, SR)]

    def norm_tiles(s_lo, s_hi):
        return [(normalise, s0, n0) for s0 in range(s_lo, s_hi, T) for n0 in tiles_n]

    def m_blocks(n0):
        return [(m_block, n0, c0) for c0 in (0, 4 * T)]

    for cp in (wq0, x0, wq1, gw, wr, x1, wq2, x2, x3, wk, wg, wu, wv, wo, wd):
        cp.start()

    wq0.wait()
    x0.wait()
    bits = pltpu.bitcast(x_v[0:16, 0:T], u32)
    st["zero"] = (bits >> 31) & (~bits >> 31)
    run([(proj_direct, n0, 0) for n0 in (0, T)], w_tiles(0, 0, XC))
    wq1.wait()
    run([(proj_direct, n0, 0) for n0 in (2 * T, 3 * T)], w_tiles(0, XC, 2 * XC))
    gw.wait()
    wr.wait()
    x1.wait()
    st["gate_w"] = gw_v[...].astype(f32).reshape(1, D)
    st["w_r"] = wr_v[...].astype(f32).reshape(1, D)
    run(proj_tiles(0, XC, 2 * XC, 2 * XC), score_tiles(0, XC))
    wq2.wait()
    run([(proj_direct, n0, s0) for n0 in range(2 * XC, D, T) for s0 in (0, XC)],
        w_tiles(0, 2 * XC, D))
    x2.wait()
    run(proj_tiles(0, 2 * XC, D), score_tiles(XC, D))
    x3.wait()
    wk.wait()
    run(proj_tiles(0, D, S - T), w_tiles(1, 0, D), score_tiles(D, S))

    run(proj_tiles(1, 0, K_SPLIT - 2 * T),
        [(route_max, s0, 2 * T) for s0 in range(0, S, 2 * T)]
        + [(route_arg, s0, T) for s0 in range(0, S, T)] + [(route_gather,)])
    run(proj_tiles(1, K_SPLIT - 2 * T, K_SPLIT), [(route_spread, k0) for k0 in tiles_n])
    wg.wait()
    wu.wait()
    up, grams = [], []
    for c in range(F // FC):
        part = [(ffn_up, c, k) for k in range(0, D, 16)]
        if c > 0:
            for i, j in enumerate(range(0, FC, ACT)):
                part.insert(8 * i + 4, (ffn_spread, c - 1, j))
        up += part + [(ffn_act,)]
    up += [(ffn_spread, F // FC - 1, j) for j in range(0, FC, ACT)]
    for n0 in tiles_n:
        for c0 in tiles_n:
            grams += [(gram, n0, c0, s0) for s0 in range(0, S, GK)]
            if n0 > 0 and c0 == 5 * T:
                grams.append((kv_block, n0 - T))
            if n0 > 0 and c0 == 7 * T:
                grams += m_blocks(n0 - T)
    run(proj_tiles(1, K_SPLIT, S) + grams[:G_EARLY], up)

    wv.wait()
    wo.wait()
    wd.wait()
    last = proj_tiles(0, S - T, S)
    run(grams[G_EARLY:] + last[:1] + [(kv_block, D - T)] + last[1:2] + m_blocks(D - T) + last[2:],
        [(ffn_down, k) for k in range(0, F, 16)] + [(ffn_finish,)],
        [(z_finish, n0) for n0 in tiles_n] + norm_tiles(0, NS))

    for s0 in range(0, S, T):
        ahead = NS + s0
        run([(final, s0, c0) for c0 in tiles_n], norm_tiles(ahead, min(ahead + T, S)))
    flush()
    for cp in stores:
        cp.wait()


@jax.jit
def pallas_gated_mix__linear_attn_block__moe_arch_mod__prompt_kernel(
    A_x: jax.Array,
    A_wqkv: jax.Array,
    A_wo: jax.Array,
    B_x: jax.Array,
    B_w_r: jax.Array,
    B_w_gate: jax.Array,
    B_w_up: jax.Array,
    B_w_down: jax.Array,
    gate_w: jax.Array,
):
    del B_x
    hbm = pl.BlockSpec(memory_space=pl.ANY)
    out = pl.pallas_call(
        _kernel,
        in_specs=[hbm] * 8,
        out_specs=hbm,
        out_shape=jax.ShapeDtypeStruct((S, D), bf16),
        scratch_shapes=[
            pltpu.VMEM((S, D), bf16),
            pltpu.VMEM((D, 3 * D), bf16),
            pltpu.VMEM((2, D // 2, D), u32),
            pltpu.VMEM((D, D), bf16),
            pltpu.VMEM((D, F), bf16),
            pltpu.VMEM((D, F), bf16),
            pltpu.VMEM((F, D), bf16),
            pltpu.VMEM((2, D // 2, S), u32),
            pltpu.VMEM((S // 2, D), u32),
            pltpu.VMEM((D // 2, T), u32),
            pltpu.VMEM((D // 2, D), u32),
            pltpu.VMEM((8, D), f32),
            pltpu.VMEM((D // 2, D), u32),
            pltpu.VMEM((S, T), f32),
            pltpu.VMEM((S, T), f32),
            pltpu.VMEM((D, T), f32),
            pltpu.VMEM((D, T), f32),
            pltpu.VMEM((F, T), f32),
            pltpu.VMEM((S, D), bf16),
            pltpu.VMEM((D,), bf16),
            pltpu.VMEM((D,), bf16),
            pltpu.SemaphoreType.DMA((15,)),
            pltpu.SemaphoreType.DMA((len(STORE_AT) + D // LAST_SPLIT,)),
        ],
        compiler_params=pltpu.CompilerParams(vmem_limit_bytes=110 * 1024 * 1024),
    )(A_x.reshape(S, D), A_wqkv, A_wo, B_w_gate, B_w_up, B_w_down, gate_w, B_w_r)
    return out.reshape(1, S, D)
```

```python
import functools

import jax
import jax.numpy as jnp
from jax import lax
import jax.experimental.pallas as pl
import jax.experimental.pallas.tpu as pltpu

S, D, F, H = 2048, 1024, 3584, 32
DH = D // H
T = 128
XC = 256
GK = 512
FC = 512
SR = 16
LAG = 4
LAG_NORM = 12
K_SPLIT = 896
G_EARLY = 56
STORE_AT = (1024, 1664, S - T)
LAST_SPLIT = 256
f32, bf16, u32 = jnp.float32, jnp.bfloat16, jnp.uint32
NT = (((1,), (1,)), ((), ()))


def _phi(t):
    return jnp.where(t > 0, t + 1.0, jnp.exp(t)) + 1e-6


def _rnd(t):
    return t.astype(bf16).astype(f32)


def _lanes(t, n):
    return jnp.concatenate([t] * n, axis=1)


def _col_bcast(row):
    n = row.shape[1]
    return jnp.concatenate(
        [jnp.broadcast_to(row[:, j:j + T], (T, T)).T for j in range(0, n, T)], axis=0)


def _ld(ref, r0, n, c0, m):
    return pltpu.bitcast(ref[r0 // 2:(r0 + n) // 2, c0:c0 + m], bf16)


def _st(ref, r0, c0, val):
    n, m = val.shape
    ref[r0 // 2:(r0 + n) // 2, c0:c0 + m] = pltpu.bitcast(val.astype(bf16), u32)


def _kernel(x_hbm, wqkv_hbm, wo_hbm, wg_hbm, wu_hbm, wd_hbm, gw_hbm, wr_hbm, out_hbm,
            x_v, w_v, wt_v, wo_v, wg_v, wu_v, wd_v, pt_v, pn_v, kv_v, gb_v, y_v, m_v, gate_v, r_v,
            z_v, xb_v, hb_v, o_v, gw_v, wr_v, sem_i, sem_o):
    def rows_in(i, r0, r1):
        return pltpu.make_async_copy(x_hbm.at[r0:r1], x_v.at[r0:r1], sem_i.at[i])

    def cols_in(i, c0, c1):
        return pltpu.make_async_copy(wqkv_hbm.at[:, c0:c1], w_v.at[:, c0:c1], sem_i.at[i])

    wq0, x0 = cols_in(0, 0, XC), rows_in(1, 0, XC)
    wq1, x1 = cols_in(2, XC, 2 * XC), rows_in(3, XC, 2 * XC)
    wq2, x2 = cols_in(4, 2 * XC, D), rows_in(5, 2 * XC, D)
    x3, wk = rows_in(6, D, S), cols_in(7, D, 2 * D)
    wg = pltpu.make_async_copy(wg_hbm, wg_v, sem_i.at[8])
    wu = pltpu.make_async_copy(wu_hbm, wu_v, sem_i.at[9])
    wv = cols_in(10, 2 * D, 3 * D)
    wo = pltpu.make_async_copy(wo_hbm, wo_v, sem_i.at[11])
    wd = pltpu.make_async_copy(wd_hbm, wd_v, sem_i.at[12])
    gw = pltpu.make_async_copy(gw_hbm, gw_v, sem_i.at[13])
    wr = pltpu.make_async_copy(wr_hbm, wr_v, sem_i.at[14])
    stores = []

    def start_store(s0, n, c0, c1):
        blk = (pl.ds(s0, n), pl.ds(c0, c1 - c0))
        stores.append(pltpu.make_async_copy(o_v.at[blk], out_hbm.at[blk], sem_o.at[len(stores)]))
        stores[-1].start()

    st = {"due": [], "go": []}

    def due(val):
        bits = pltpu.bitcast(val, u32)
        st["due"] += [bits[r:r + 8, c:c + T] for r in range(0, bits.shape[0], 8)
                      for c in range(0, bits.shape[1], T)]

    def paced(rhs):
        if "chain" in st:
            due(st.pop("chain"))
        if not st["due"]:
            return rhs
        tok = functools.reduce(jnp.bitwise_or, st["due"]) & st["zero"]
        st["due"] = []
        bits = pltpu.bitcast(rhs, u32)
        top = bits[0:8, 0:T] | tok
        return pltpu.bitcast(
            jnp.concatenate([jnp.concatenate([top, bits[0:8, T:]], axis=1)
                             if bits.shape[1] > T else top, bits[8:]], axis=0), bf16)

    def gated(val, lag=LAG):
        if len(st["go"]) < lag:
            return val
        bits = pltpu.bitcast(val, u32)
        go = jnp.tile(st["go"][-lag], (bits.shape[0] // 8, bits.shape[1] // T))
        return pltpu.bitcast(bits | go, val.dtype)

    def flush():
        st.pop("tail", lambda: None)()

    def issued(acc, tail):
        flush()
        st["tail"] = tail
        st["go"].append(pltpu.bitcast(acc[0:8, 0:T], u32) & st["zero"])

    def run(pieces, *lanes):
        n, done = len(pieces), [0] * len(lanes)
        for p, (fn, *args) in enumerate(pieces):
            fn(*args)
            for li, lane in enumerate(lanes):
                upto = -(-len(lane) * (p + 1) // n)
                for side, *side_args in lane[done[li]:upto]:
                    side(*side_args)
                done[li] = upto
        st["due"] = []
        st.pop("chain", None)

    def transpose_w(t, c0, k0):
        wt = gated(w_v[k0:k0 + XC, t * D + c0:t * D + c0 + T]).T
        _st(wt_v.at[t], c0, k0, wt)
        due(wt)

    def scores(s0):
        xs = gated(x_v[s0:s0 + SR, :]).astype(f32)
        gl = jnp.sum(xs * st["gate_w"], axis=1, keepdims=True)
        gate = jax.nn.sigmoid(jnp.broadcast_to(gl, (SR, T)))
        gate_v[s0:s0 + SR, :] = gate
        r = jnp.sum(xs * st["w_r"], axis=1, keepdims=True)
        r = _rnd(jnp.broadcast_to(r, (SR, T)))
        r_v[s0:s0 + SR, :] = r
        due(gate)
        due(r)

    def route_max(s0, n):
        m = jnp.max(gated(r_v[s0:s0 + n, :]).reshape(n // 8, 8, T), axis=0)
        st["m8"] = m if s0 == 0 else jnp.maximum(st["m8"], m)
        if s0 + n == S:
            st["r_max"] = jnp.max(st["m8"], axis=0, keepdims=True)
        due(st["m8"])

    def route_arg(s0, n):
        tok = lax.broadcasted_iota(jnp.int32, (n, T), 0) + s0
        cand = jnp.where(gated(r_v[s0:s0 + n, :]) == st["r_max"], tok, S - 1)
        m = jnp.min(cand.reshape(n // 8, 8, T), axis=0)
        st["i8"] = m if s0 == 0 else jnp.minimum(st["i8"], m)
        due(st["i8"])

    def route_gather():
        idx = jnp.min(st["i8"])
        base = pl.multiple_of((idx // 16) * 16, 16)
        grp = x_v[pl.ds(base, 16), :].astype(f32)
        sel = lax.broadcasted_iota(jnp.int32, (16, 1), 0) == idx - base
        st["x_sel"] = jnp.sum(jnp.where(sel, grp, 0.0), axis=0, keepdims=True)
        st["idx"] = idx

    def route_spread(k0):
        xb = _col_bcast(st["x_sel"][:, k0:k0 + T])
        xb_v[k0:k0 + T, :] = xb
        due(xb)

    def accumulate(part, first):
        part = part if first else y_v[...] + part
        y_v[...] = part
        st["chain"] = part

    def ffn_up(c, k):
        cols = slice(c * FC, (c + 1) * FC)
        xk = _lanes(gated(xb_v[k:k + 16, :]), FC // T)
        pg = wg_v[k:k + 16, cols].astype(f32) * xk
        pu = wu_v[k:k + 16, cols].astype(f32) * xk
        pg, pu = pg[:8] + pg[8:], pu[:8] + pu[8:]
        accumulate(jnp.concatenate([pg, pu], axis=1), k == 0)

    def ffn_act():
        hg = _rnd(jnp.sum(y_v[:, :FC], axis=0, keepdims=True))
        hu = _rnd(jnp.sum(y_v[:, FC:], axis=0, keepdims=True))
        st["h"] = _rnd(_rnd(hg * jax.nn.sigmoid(hg)) * hu)

    def ffn_spread(c):
        hb = _col_bcast(st["h"])
        hb_v[c * FC:(c + 1) * FC, :] = hb
        due(hb)

    def ffn_down(k):
        py = wd_v[k:k + 16, :].astype(f32) * _lanes(gated(hb_v[k:k + 16, :]), D // T)
        accumulate(py[:8] + py[8:], k == 0)

    def ffn_finish():
        y = _rnd(_rnd(jnp.sum(y_v[...], axis=0, keepdims=True))
                 * _lanes(_rnd(jax.nn.sigmoid(st["r_max"])), D // T))
        y_v[...] = jnp.broadcast_to(y, (8, D))

    def z_finish(n0):
        z = _rnd(jnp.sum(z_v[n0:n0 + T, :], axis=1, keepdims=True))
        z = jnp.broadcast_to(z, (T, T))
        z_v[n0:n0 + T, :] = z
        due(z)

    def normalise(s0, n0):
        pq = gated(_ld(pt_v.at[0], n0, T, s0, T), LAG_NORM).astype(f32).reshape(T // DH, DH, T)
        zz = z_v[n0:n0 + T, :].reshape(T // DH, DH, T)
        den = jnp.sum(pq * zz, axis=1, keepdims=True) + 1e-6
        pn = (pq * (1.0 / den)).reshape(T, T).astype(bf16).T
        _st(pn_v, s0, n0, pn)
        due(pn)

    def proj(t, n0, s0):
        lhs = wt_v[t, n0 // 2:(n0 + T) // 2, :] | jnp.tile(st["zero"], (T // 16, D // T))
        acc = lax.dot_general(pltpu.bitcast(lhs, bf16), paced(x_v[s0:s0 + T, :]), NT,
                              preferred_element_type=f32)

        def tail():
            p = _phi(acc)
            _st(pt_v.at[t], n0, s0, p)
            if t == 1:
                z_v[n0:n0 + T, :] = p if s0 == 0 else z_v[n0:n0 + T, :] + p
        issued(acc, tail)

    def proj_direct(n0, s0):
        acc = jnp.dot(x_v[s0:s0 + XC, :], paced(w_v[:, n0:n0 + T]), preferred_element_type=f32)
        issued(acc, lambda: _st(pt_v.at[0], n0, s0, _phi(acc).T))

    def gram(n0, c0, s0):
        acc = jnp.dot(_ld(pt_v.at[1], n0, T, s0, GK), paced(x_v[s0:s0 + GK, c0:c0 + T]),
                      preferred_element_type=f32)

        def tail():
            st["g"] = acc if s0 == 0 else st["g"] + acc
            if s0 + GK == S:
                _st(gb_v, n0, c0, st["g"])
        issued(acc, tail)

    def kv_block(n0):
        kv = jnp.dot(_ld(gb_v, n0, T, 0, D), w_v[:, 2 * D + n0:2 * D + n0 + T],
                     preferred_element_type=f32)
        same_head = (lax.broadcasted_iota(jnp.int32, (T, T), 0) // DH
                     == lax.broadcasted_iota(jnp.int32, (T, T), 1) // DH)
        _st(kv_v, n0, 0, jnp.where(same_head, kv, 0.0))

    def m_block(n0, c0):
        _st(m_v, n0, c0, jnp.dot(_ld(kv_v, n0, T, 0, T), wo_v[n0:n0 + T, c0:c0 + 4 * T],
                                 preferred_element_type=f32))

    def final(s0, c0):
        a = jnp.dot(_ld(pn_v, s0, T, 0, D), paced(_ld(m_v, 0, D, c0, T)),
                    preferred_element_type=f32)

        def tail():
            rows, cols = slice(s0, s0 + T), slice(c0, c0 + T)
            gate = gate_v[rows, :]
            xs = x_v[rows, cols].astype(f32)
            hit = lax.broadcasted_iota(jnp.int32, (T, T), 0) == st["idx"] - s0
            y = jnp.broadcast_to(y_v[0:1, cols], (T, T))
            b = xs + (xs * 0.0 + jnp.where(hit, y, 0.0))
            o_v[rows, cols] = (gate * a + (1.0 - gate) * b).astype(bf16)
            if s0 + T == S:
                if (c0 + T) % LAST_SPLIT == 0:
                    start_store(s0, T, c0 + T - LAST_SPLIT, c0 + T)
            elif c0 + T == D and s0 + T in STORE_AT:
                r0 = ((0,) + STORE_AT)[STORE_AT.index(s0 + T)]
                start_store(r0, s0 + T - r0, 0, D)
        issued(a, tail)

    tiles_n = range(0, D, T)

    def proj_tiles(t, s_lo, s_hi, n_hi=D):
        return [(proj, t, n0, s0) for s0 in range(s_lo, s_hi, T) for n0 in range(0, n_hi, T)]

    def w_tiles(t, n_lo, n_hi):
        return [(transpose_w, t, n0, k0) for n0 in range(n_lo, n_hi, T) for k0 in range(0, D, XC)]

    def score_tiles(s_lo, s_hi):
        return [(scores, s0) for s0 in range(s_lo, s_hi, SR)]

    def norm_tiles(s_lo, s_hi):
        return [(normalise, s0, n0) for s0 in range(s_lo, s_hi, T) for n0 in tiles_n]

    def m_blocks(n0):
        return [(m_block, n0, c0) for c0 in (0, 4 * T)]

    for cp in (wq0, x0, wq1, gw, wr, x1, wq2, x2, x3, wk, wg, wu, wv, wo, wd):
        cp.start()

    wq0.wait()
    x0.wait()
    bits = pltpu.bitcast(x_v[0:16, 0:T], u32)
    st["zero"] = (bits >> 31) & (~bits >> 31)
    run([(proj_direct, n0, 0) for n0 in (0, T)], w_tiles(0, 0, XC))
    wq1.wait()
    run([(proj_direct, n0, 0) for n0 in (2 * T, 3 * T)], w_tiles(0, XC, 2 * XC))
    gw.wait()
    wr.wait()
    x1.wait()
    st["gate_w"] = gw_v[...].astype(f32).reshape(1, D)
    st["w_r"] = wr_v[...].astype(f32).reshape(1, D)
    run(proj_tiles(0, XC, 2 * XC, 2 * XC), score_tiles(0, XC))
    wq2.wait()
    run([(proj_direct, n0, s0) for n0 in range(2 * XC, D, T) for s0 in (0, XC)],
        w_tiles(0, 2 * XC, D))
    x2.wait()
    run(proj_tiles(0, 2 * XC, D), score_tiles(XC, D))
    x3.wait()
    wk.wait()
    run(proj_tiles(0, D, S - T), w_tiles(1, 0, D), score_tiles(D, S))

    run(proj_tiles(1, 0, K_SPLIT - 2 * T),
        [(route_max, s0, 2 * T) for s0 in range(0, S, 2 * T)]
        + [(route_arg, s0, T) for s0 in range(0, S, T)] + [(route_gather,)])
    run(proj_tiles(1, K_SPLIT - 2 * T, K_SPLIT), [(route_spread, k0) for k0 in tiles_n])
    wg.wait()
    wu.wait()
    up, grams = [], []
    for c in range(F // FC):
        part = [(ffn_up, c, k) for k in range(0, D, 16)]
        if c > 0:
            part.insert(4, (ffn_spread, c - 1))
        up += part + [(ffn_act,)]
    up.append((ffn_spread, F // FC - 1))
    for n0 in tiles_n:
        for c0 in tiles_n:
            grams += [(gram, n0, c0, s0) for s0 in range(0, S, GK)]
            if n0 > 0 and c0 == 5 * T:
                grams.append((kv_block, n0 - T))
            if n0 > 0 and c0 == 7 * T:
                grams += m_blocks(n0 - T)
    run(proj_tiles(1, K_SPLIT, S) + grams[:G_EARLY], up)

    wv.wait()
    wo.wait()
    wd.wait()
    last = proj_tiles(0, S - T, S)
    run(grams[G_EARLY:] + last[:1] + [(kv_block, D - T)] + last[1:2] + m_blocks(D - T) + last[2:],
        [(ffn_down, k) for k in range(0, F, 16)] + [(ffn_finish,)],
        [(z_finish, n0) for n0 in tiles_n] + norm_tiles(0, S - 2 * T))

    for s0 in range(0, S, T):
        ahead = S - 2 * T + s0
        run([(final, s0, c0) for c0 in tiles_n], norm_tiles(ahead, min(ahead + T, S)))
    flush()
    for cp in stores:
        cp.wait()


@jax.jit
def pallas_gated_mix__linear_attn_block__moe_arch_mod__prompt_kernel(
    A_x: jax.Array,
    A_wqkv: jax.Array,
    A_wo: jax.Array,
    B_x: jax.Array,
    B_w_r: jax.Array,
    B_w_gate: jax.Array,
    B_w_up: jax.Array,
    B_w_down: jax.Array,
    gate_w: jax.Array,
):
    del B_x
    hbm = pl.BlockSpec(memory_space=pl.ANY)
    out = pl.pallas_call(
        _kernel,
        in_specs=[hbm] * 8,
        out_specs=hbm,
        out_shape=jax.ShapeDtypeStruct((S, D), bf16),
        scratch_shapes=[
            pltpu.VMEM((S, D), bf16),
            pltpu.VMEM((D, 3 * D), bf16),
            pltpu.VMEM((2, D // 2, D), u32),
            pltpu.VMEM((D, D), bf16),
            pltpu.VMEM((D, F), bf16),
            pltpu.VMEM((D, F), bf16),
            pltpu.VMEM((F, D), bf16),
            pltpu.VMEM((2, D // 2, S), u32),
            pltpu.VMEM((S // 2, D), u32),
            pltpu.VMEM((D // 2, T), u32),
            pltpu.VMEM((D // 2, D), u32),
            pltpu.VMEM((8, D), f32),
            pltpu.VMEM((D // 2, D), u32),
            pltpu.VMEM((S, T), f32),
            pltpu.VMEM((S, T), f32),
            pltpu.VMEM((D, T), f32),
            pltpu.VMEM((D, T), f32),
            pltpu.VMEM((F, T), f32),
            pltpu.VMEM((S, D), bf16),
            pltpu.VMEM((D,), bf16),
            pltpu.VMEM((D,), bf16),
            pltpu.SemaphoreType.DMA((15,)),
            pltpu.SemaphoreType.DMA((len(STORE_AT) + D // LAST_SPLIT,)),
        ],
        compiler_params=pltpu.CompilerParams(vmem_limit_bytes=110 * 1024 * 1024),
    )(A_x.reshape(S, D), A_wqkv, A_wo, B_w_gate, B_w_up, B_w_down, gate_w, B_w_r)
    return out.reshape(1, S, D)
```

```python
import functools

import jax
import jax.numpy as jnp
from jax import lax
import jax.experimental.pallas as pl
import jax.experimental.pallas.tpu as pltpu

S, D, F, H = 2048, 1024, 3584, 32
DH = D // H
T = 128
XC = 256
GK = 512
FC = 512
SR = 16
LAG = 4
LAG_NORM = 8
G_EARLY = 48
N_AHEAD = 512
STORE_AT = (1024, 1664, S - T)
LAST_SPLIT = 256
f32, bf16, u32 = jnp.float32, jnp.bfloat16, jnp.uint32
NT = (((1,), (1,)), ((), ()))


def _phi(t):
    return jnp.where(t > 0, t + 1.0, jnp.exp(t)) + 1e-6


def _rnd(t):
    return t.astype(bf16).astype(f32)


def _lanes(t, n):
    return jnp.concatenate([t] * n, axis=1)


def _col_bcast(row):
    n = row.shape[1]
    return jnp.concatenate(
        [jnp.broadcast_to(row[:, j:j + T], (T, T)).T for j in range(0, n, T)], axis=0)


def _ld(ref, r0, n, c0, m):
    return pltpu.bitcast(ref[r0 // 2:(r0 + n) // 2, c0:c0 + m], bf16)


def _st(ref, r0, c0, val):
    n, m = val.shape
    ref[r0 // 2:(r0 + n) // 2, c0:c0 + m] = pltpu.bitcast(val.astype(bf16), u32)


def _kernel(x_hbm, wqkv_hbm, wo_hbm, wg_hbm, wu_hbm, wd_hbm, gw_hbm, wr_hbm, out_hbm,
            x_v, w_v, wt_v, wo_v, wg_v, wu_v, wd_v, pt_v, pn_v, kv_v, gb_v, y_v, m_v, gate_v, r_v,
            z_v, xb_v, hb_v, o_v, gw_v, wr_v, sem_i, sem_o):
    def rows_in(i, r0, r1):
        return pltpu.make_async_copy(x_hbm.at[r0:r1], x_v.at[r0:r1], sem_i.at[i])

    def cols_in(i, c0, c1):
        return pltpu.make_async_copy(wqkv_hbm.at[:, c0:c1], w_v.at[:, c0:c1], sem_i.at[i])

    wq0, x0 = cols_in(0, 0, XC), rows_in(1, 0, XC)
    wq1, x1 = cols_in(2, XC, 2 * XC), rows_in(3, XC, 2 * XC)
    wq2, x2 = cols_in(4, 2 * XC, D), rows_in(5, 2 * XC, D)
    x3, wk = rows_in(6, D, S), cols_in(7, D, 2 * D)
    wg = pltpu.make_async_copy(wg_hbm, wg_v, sem_i.at[8])
    wu = pltpu.make_async_copy(wu_hbm, wu_v, sem_i.at[9])
    wv = cols_in(10, 2 * D, 3 * D)
    wo = pltpu.make_async_copy(wo_hbm, wo_v, sem_i.at[11])
    wd = pltpu.make_async_copy(wd_hbm, wd_v, sem_i.at[12])
    gw = pltpu.make_async_copy(gw_hbm, gw_v, sem_i.at[13])
    wr = pltpu.make_async_copy(wr_hbm, wr_v, sem_i.at[14])
    stores = []

    def start_store(s0, n, c0, c1):
        blk = (pl.ds(s0, n), pl.ds(c0, c1 - c0))
        stores.append(pltpu.make_async_copy(o_v.at[blk], out_hbm.at[blk], sem_o.at[len(stores)]))
        stores[-1].start()

    st = {"due": [], "go": []}

    def due(val):
        bits = pltpu.bitcast(val, u32)
        st["due"] += [bits[r:r + 8, c:c + T] for r in range(0, bits.shape[0], 8)
                      for c in range(0, bits.shape[1], T)]

    def paced(rhs):
        if "chain" in st:
            due(st.pop("chain"))
        if not st["due"]:
            return rhs
        tok = functools.reduce(jnp.bitwise_or, st["due"]) & st["zero"]
        st["due"] = []
        bits = pltpu.bitcast(rhs, u32)
        top = bits[0:8, 0:T] | tok
        return pltpu.bitcast(
            jnp.concatenate([jnp.concatenate([top, bits[0:8, T:]], axis=1)
                             if bits.shape[1] > T else top, bits[8:]], axis=0), bf16)

    def gated(val, lag=LAG):
        if len(st["go"]) < lag:
            return val
        bits = pltpu.bitcast(val, u32)
        go = jnp.tile(st["go"][-lag], (bits.shape[0] // 8, bits.shape[1] // T))
        return pltpu.bitcast(bits | go, val.dtype)

    def flush():
        st.pop("tail", lambda: None)()

    def issued(acc, tail):
        flush()
        st["tail"] = tail
        st["go"].append(pltpu.bitcast(acc[0:8, 0:T], u32) & st["zero"])

    def run(pieces, *lanes):
        n, done = len(pieces), [0] * len(lanes)
        for p, (fn, *args) in enumerate(pieces):
            fn(*args)
            for li, lane in enumerate(lanes):
                upto = -(-len(lane) * (p + 1) // n)
                for side, *side_args in lane[done[li]:upto]:
                    side(*side_args)
                done[li] = upto
        st["due"] = []
        st.pop("chain", None)

    def transpose_w(t, c0, k0):
        wt = gated(w_v[k0:k0 + XC, t * D + c0:t * D + c0 + T]).T
        _st(wt_v.at[t], c0, k0, wt)
        due(wt)

    def scores(s0):
        xs = gated(x_v[s0:s0 + SR, :]).astype(f32)
        gl = jnp.sum(xs * st["gate_w"], axis=1, keepdims=True)
        gate = jax.nn.sigmoid(jnp.broadcast_to(gl, (SR, T)))
        gate_v[s0:s0 + SR, :] = gate
        r = jnp.sum(xs * st["w_r"], axis=1, keepdims=True)
        r = _rnd(jnp.broadcast_to(r, (SR, T)))
        r_v[s0:s0 + SR, :] = r
        due(gate)
        due(r)

    def route_max(s0, n):
        m = jnp.max(gated(r_v[s0:s0 + n, :]).reshape(n // 8, 8, T), axis=0)
        st["m8"] = m if s0 == 0 else jnp.maximum(st["m8"], m)
        if s0 + n == S:
            st["r_max"] = jnp.max(st["m8"], axis=0, keepdims=True)
        due(st["m8"])

    def route_arg(s0, n):
        tok = lax.broadcasted_iota(jnp.int32, (n, T), 0) + s0
        cand = jnp.where(gated(r_v[s0:s0 + n, :]) == st["r_max"], tok, S - 1)
        m = jnp.min(cand.reshape(n // 8, 8, T), axis=0)
        st["i8"] = m if s0 == 0 else jnp.minimum(st["i8"], m)
        due(st["i8"])

    def route_gather():
        idx = jnp.min(st["i8"])
        base = pl.multiple_of((idx // 16) * 16, 16)
        grp = x_v[pl.ds(base, 16), :].astype(f32)
        sel = lax.broadcasted_iota(jnp.int32, (16, 1), 0) == idx - base
        st["x_sel"] = jnp.sum(jnp.where(sel, grp, 0.0), axis=0, keepdims=True)
        st["idx"] = idx

    def route_spread(k0):
        xb = _col_bcast(st["x_sel"][:, k0:k0 + T])
        xb_v[k0:k0 + T, :] = xb
        due(xb)

    def accumulate(part, first):
        part = part if first else y_v[...] + part
        y_v[...] = part
        st["chain"] = part

    def ffn_up(c, k):
        cols = slice(c * FC, (c + 1) * FC)
        xk = _lanes(gated(xb_v[k:k + 16, :]), FC // T)
        pg = wg_v[k:k + 16, cols].astype(f32) * xk
        pu = wu_v[k:k + 16, cols].astype(f32) * xk
        pg, pu = pg[:8] + pg[8:], pu[:8] + pu[8:]
        accumulate(jnp.concatenate([pg, pu], axis=1), k == 0)

    def ffn_act():
        hg = _rnd(jnp.sum(y_v[:, :FC], axis=0, keepdims=True))
        hu = _rnd(jnp.sum(y_v[:, FC:], axis=0, keepdims=True))
        st["h"] = _rnd(_rnd(hg * jax.nn.sigmoid(hg)) * hu)

    def ffn_spread(c):
        hb = _col_bcast(st["h"])
        hb_v[c * FC:(c + 1) * FC, :] = hb
        due(hb)

    def ffn_down(k):
        py = wd_v[k:k + 16, :].astype(f32) * _lanes(gated(hb_v[k:k + 16, :], LAG + 1), D // T)
        accumulate(py[:8] + py[8:], k == 0)

    def ffn_finish():
        y = _rnd(_rnd(jnp.sum(y_v[...], axis=0, keepdims=True))
                 * _lanes(_rnd(jax.nn.sigmoid(st["r_max"])), D // T))
        y_v[...] = jnp.broadcast_to(y, (8, D))

    def z_finish(n0):
        z = _rnd(jnp.sum(z_v[n0:n0 + T, :], axis=1, keepdims=True))
        z = jnp.broadcast_to(z, (T, T))
        z_v[n0:n0 + T, :] = z
        due(z)

    def normalise(s0, n0):
        pq = gated(_ld(pt_v.at[0], n0, T, s0, T), LAG_NORM).astype(f32).reshape(T // DH, DH, T)
        zz = z_v[n0:n0 + T, :].reshape(T // DH, DH, T)
        den = jnp.sum(pq * zz, axis=1, keepdims=True) + 1e-6
        pn = (pq * (1.0 / den)).reshape(T, T).astype(bf16).T
        _st(pn_v, s0, n0, pn)
        due(pn)

    def proj(t, n0, s0):
        lhs = wt_v[t, n0 // 2:(n0 + T) // 2, :] | jnp.tile(st["zero"], (T // 16, D // T))
        acc = lax.dot_general(pltpu.bitcast(lhs, bf16), paced(x_v[s0:s0 + T, :]), NT,
                              preferred_element_type=f32)

        def tail():
            p = _phi(acc)
            _st(pt_v.at[t], n0, s0, p)
            if t == 1:
                z_v[n0:n0 + T, :] = p if s0 == 0 else z_v[n0:n0 + T, :] + p
        issued(acc, tail)

    def proj_direct(n0, s0):
        acc = jnp.dot(x_v[s0:s0 + XC, :], paced(w_v[:, n0:n0 + T]), preferred_element_type=f32)
        issued(acc, lambda: _st(pt_v.at[0], n0, s0, _phi(acc).T))

    def gram(n0, c0, s0):
        acc = jnp.dot(_ld(pt_v.at[1], n0, T, s0, GK), paced(x_v[s0:s0 + GK, c0:c0 + T]),
                      preferred_element_type=f32)

        def tail():
            st["g"] = acc if s0 == 0 else st["g"] + acc
            if s0 + GK == S:
                _st(gb_v, n0, c0, st["g"])
        issued(acc, tail)

    def kv_block(n0):
        kv = jnp.dot(_ld(gb_v, n0, T, 0, D), w_v[:, 2 * D + n0:2 * D + n0 + T],
                     preferred_element_type=f32)
        same_head = (lax.broadcasted_iota(jnp.int32, (T, T), 0) // DH
                     == lax.broadcasted_iota(jnp.int32, (T, T), 1) // DH)
        _st(kv_v, n0, 0, jnp.where(same_head, kv, 0.0))

    def m_block(n0, c0):
        _st(m_v, n0, c0, jnp.dot(_ld(kv_v, n0, T, 0, T), wo_v[n0:n0 + T, c0:c0 + 4 * T],
                                 preferred_element_type=f32))

    def final(s0, c0):
        a = jnp.dot(_ld(pn_v, s0, T, 0, D), paced(_ld(m_v, 0, D, c0, T)),
                    preferred_element_type=f32)

        def tail():
            rows, cols = slice(s0, s0 + T), slice(c0, c0 + T)
            gate = gate_v[rows, :]
            xs = x_v[rows, cols].astype(f32)
            hit = lax.broadcasted_iota(jnp.int32, (T, T), 0) == st["idx"] - s0
            y = jnp.broadcast_to(y_v[0:1, cols], (T, T))
            b = xs + (xs * 0.0 + jnp.where(hit, y, 0.0))
            o_v[rows, cols] = (gate * a + (1.0 - gate) * b).astype(bf16)
            if s0 + T == S:
                if (c0 + T) % LAST_SPLIT == 0:
                    start_store(s0, T, c0 + T - LAST_SPLIT, c0 + T)
            elif c0 + T == D and s0 + T in STORE_AT:
                r0 = ((0,) + STORE_AT)[STORE_AT.index(s0 + T)]
                start_store(r0, s0 + T - r0, 0, D)
        issued(a, tail)

    tiles_n = range(0, D, T)

    def proj_tiles(t, s_lo, s_hi, n_hi=D):
        return [(proj, t, n0, s0) for s0 in range(s_lo, s_hi, T) for n0 in range(0, n_hi, T)]

    def w_tiles(t, n_lo, n_hi):
        return [(transpose_w, t, n0, k0) for n0 in range(n_lo, n_hi, T) for k0 in range(0, D, XC)]

    def score_tiles(s_lo, s_hi):
        return [(scores, s0) for s0 in range(s_lo, s_hi, SR)]

    def norm_tiles(s_lo, s_hi):
        return [(normalise, s0, n0) for s0 in range(s_lo, s_hi, T) for n0 in tiles_n]

    def m_blocks(n0):
        return [(m_block, n0, c0) for c0 in (0, 4 * T)]

    for cp in (wq0, x0, wq1, gw, wr, x1, wq2, x2, x3, wk, wg, wu, wv, wo, wd):
        cp.start()

    wq0.wait()
    x0.wait()
    bits = pltpu.bitcast(x_v[0:16, 0:T], u32)
    st["zero"] = (bits >> 31) & (~bits >> 31)
    run([(proj_direct, n0, 0) for n0 in (0, T)], w_tiles(0, 0, XC))
    wq1.wait()
    run([(proj_direct, n0, 0) for n0 in (2 * T, 3 * T)], w_tiles(0, XC, 2 * XC))
    gw.wait()
    wr.wait()
    x1.wait()
    st["gate_w"] = gw_v[...].astype(f32).reshape(1, D)
    st["w_r"] = wr_v[...].astype(f32).reshape(1, D)
    run(proj_tiles(0, XC, 2 * XC, 2 * XC), score_tiles(0, XC))
    wq2.wait()
    run([(proj_direct, n0, s0) for n0 in range(2 * XC, D, T) for s0 in (0, XC)],
        w_tiles(0, 2 * XC, D))
    x2.wait()
    run(proj_tiles(0, 2 * XC, D), score_tiles(XC, 3 * XC))
    x3.wait()
    wk.wait()
    run(proj_tiles(0, D, S - T), w_tiles(1, 0, D), score_tiles(3 * XC, 9 * T))

    run(proj_tiles(1, 0, D), score_tiles(9 * T, S))
    run(proj_tiles(1, D, S - 2 * T),
        [(route_max, s0, 2 * T) for s0 in range(0, S, 2 * T)]
        + [(route_arg, s0, T) for s0 in range(0, S, T)] + [(route_gather,)])
    run(proj_tiles(1, S - 2 * T, S), [(route_spread, k0) for k0 in tiles_n])

    ffn, grams = [], []
    for c in range(F // FC):
        part = [(ffn_up, c, k) for k in range(0, D, 16)]
        if c > 0:
            part.insert(4, (ffn_spread, c - 1))
        ffn += part + [(ffn_act,)]
    ffn += [(ffn_spread, F // FC - 1)] + [(ffn_down, k) for k in range(0, F, 16)] + [(ffn_finish,)]
    for n0 in tiles_n:
        for c0 in tiles_n:
            grams += [(gram, n0, c0, s0) for s0 in range(0, S, GK)]
            if n0 > 0 and c0 == 5 * T:
                grams.append((kv_block, n0 - T))
            if n0 > 0 and c0 == 7 * T:
                grams += m_blocks(n0 - T)
    run(grams[:G_EARLY], [(z_finish, n0) for n0 in tiles_n] + norm_tiles(0, N_AHEAD))
    for cp in (wg, wu, wv, wo, wd):
        cp.wait()
    last = proj_tiles(0, S - T, S)
    run(grams[G_EARLY:] + last[:1] + [(kv_block, D - T)] + last[1:2] + m_blocks(D - T) + last[2:],
        ffn)

    for s0 in range(0, S, T):
        run([(final, s0, c0) for c0 in tiles_n],
            norm_tiles(s0 + N_AHEAD, min(s0 + N_AHEAD + T, S)))
    flush()
    for cp in stores:
        cp.wait()


@jax.jit
def pallas_gated_mix__linear_attn_block__moe_arch_mod__prompt_kernel(
    A_x: jax.Array,
    A_wqkv: jax.Array,
    A_wo: jax.Array,
    B_x: jax.Array,
    B_w_r: jax.Array,
    B_w_gate: jax.Array,
    B_w_up: jax.Array,
    B_w_down: jax.Array,
    gate_w: jax.Array,
):
    del B_x
    hbm = pl.BlockSpec(memory_space=pl.ANY)
    out = pl.pallas_call(
        _kernel,
        in_specs=[hbm] * 8,
        out_specs=hbm,
        out_shape=jax.ShapeDtypeStruct((S, D), bf16),
        scratch_shapes=[
            pltpu.VMEM((S, D), bf16),
            pltpu.VMEM((D, 3 * D), bf16),
            pltpu.VMEM((2, D // 2, D), u32),
            pltpu.VMEM((D, D), bf16),
            pltpu.VMEM((D, F), bf16),
            pltpu.VMEM((D, F), bf16),
            pltpu.VMEM((F, D), bf16),
            pltpu.VMEM((2, D // 2, S), u32),
            pltpu.VMEM((S // 2, D), u32),
            pltpu.VMEM((D // 2, T), u32),
            pltpu.VMEM((D // 2, D), u32),
            pltpu.VMEM((8, D), f32),
            pltpu.VMEM((D // 2, D), u32),
            pltpu.VMEM((S, T), f32),
            pltpu.VMEM((S, T), f32),
            pltpu.VMEM((D, T), f32),
            pltpu.VMEM((D, T), f32),
            pltpu.VMEM((F, T), f32),
            pltpu.VMEM((S, D), bf16),
            pltpu.VMEM((D,), bf16),
            pltpu.VMEM((D,), bf16),
            pltpu.SemaphoreType.DMA((15,)),
            pltpu.SemaphoreType.DMA((len(STORE_AT) + D // LAST_SPLIT,)),
        ],
        compiler_params=pltpu.CompilerParams(vmem_limit_bytes=110 * 1024 * 1024),
    )(A_x.reshape(S, D), A_wqkv, A_wo, B_w_gate, B_w_up, B_w_down, gate_w, B_w_r)
    return out.reshape(1, S, D)
```
